```python
import os as _os
_os.environ.setdefault("JAX_PLATFORMS", "cpu")
import jax
import jax.numpy as jnp

def _softmax(x, axis=-1):
    return jax.nn.softmax(x, axis=axis)
def _gelu(x):
    return jax.nn.gelu(x, approximate=True)
def _silu(x):
    return jax.nn.silu(x)
def _sigmoid(x):
    return jax.nn.sigmoid(x)
def _layernorm(x, axis=-1, eps=1e-5):
    m = jnp.mean(x, axis=axis, keepdims=True)
    v = jnp.var(x, axis=axis, keepdims=True)
    return (x - m) / jnp.sqrt(v + eps)
def _scatter_add(tgt, idx, src, axis=0):
    return tgt.at[idx].add(src)
def _segment_sum(src, seg, n):
    return jax.ops.segment_sum(src, seg, n)
class _Rng:
    def __init__(self, key):
        self._k = key
    def _next(self):
        self._k, sub = jax.random.split(self._k)
        return sub
    def normal(self, shape):
        return jax.random.normal(self._next(), shape, dtype=jnp.bfloat16)
    def randint(self, lo, hi, shape):
        return jax.random.randint(self._next(), shape, lo, hi, dtype=jnp.int32)
    def uniform(self, shape, lo=0.0, hi=1.0):
        return jax.random.uniform(self._next(), shape, jnp.bfloat16, lo, hi)
    def permutation(self, n):
        return jax.random.permutation(self._next(), n)


kernel_name = 'concat_heads__sliding_block__ssm_conv_s4__prompt'

def setup_inputs():
    _rng = _Rng(jax.random.key(int.from_bytes(__import__("os").urandom(4), "little")))
    _w = (lambda a: (lambda t: t.astype(jnp.bfloat16) if jnp.issubdtype(t.dtype, jnp.floating) else t)(jnp.asarray(a)))
    def _A_setup():
        B, S, D = 1, 2048, 512
        return {
            "x": _w((lambda *s: _rng.normal(s) * 0.2)(B, S, D)),
            "wqkv": _w((lambda *s: _rng.normal(s) * 0.2)(D, 3 * D)),
            "wo": _w((lambda *s: _rng.normal(s) * 0.05)(D, D)),
        }
    _A_in = _A_setup()

    def _B_setup():
        B, L, D, N = 1, 2048, 512, 128
        A_re = -jnp.exp((lambda *s: _rng.normal(s) * 0.8)(D, N))
        A_im = jnp.pi * (lambda *s: _rng.normal(s) * 0.8)(D, N)
        B_re = (lambda *s: _rng.normal(s) * 0.8)(D, N)
        B_im = (lambda *s: _rng.normal(s) * 0.8)(D, N)
        C_re = (lambda *s: _rng.normal(s) * 0.8)(D, N)
        C_im = (lambda *s: _rng.normal(s) * 0.8)(D, N)
        log_dt = (lambda *s: _rng.normal(s) * 0.8)(D) * 0.5 - 4.0
        Dskip = (lambda *s: _rng.normal(s) * 0.05)(D)
        return {
            "u": _w((lambda *s: _rng.normal(s) * 0.05)(B, L, D)),
            "A_re": _w(A_re),
            "A_im": _w(A_im),
            "B_re": _w(B_re),
            "B_im": _w(B_im),
            "C_re": _w(C_re),
            "C_im": _w(C_im),
            "log_dt": _w(log_dt),
            "Dskip": _w(Dskip),
        }
    _B_in = _B_setup()

    return {
        "A_x": _A_in["x"],
        "A_wqkv": _A_in["wqkv"],
        "A_wo": _A_in["wo"],
        "B_u": _B_in["u"],
        "B_A_re": _B_in["A_re"],
        "B_A_im": _B_in["A_im"],
        "B_B_re": _B_in["B_re"],
        "B_B_im": _B_in["B_im"],
        "B_C_re": _B_in["C_re"],
        "B_C_im": _B_in["C_im"],
        "B_log_dt": _B_in["log_dt"],
        "B_Dskip": _B_in["Dskip"],
    }

def reference(A_x, A_wqkv, A_wo, B_u, B_A_re, B_A_im, B_B_re, B_B_im, B_C_re, B_C_im, B_log_dt, B_Dskip):
    def _A_ref(x, wqkv, wo):
        B, S, D = x.shape
        H = 32; Dh = D // H; W = 256
        qkv = (lambda x, *d: x.transpose(*d))((x @ wqkv).reshape(B, S, 3, H, Dh), 2, 0, 3, 1, 4)
        q, k, v = qkv[0], qkv[1], qkv[2]
        scores = jnp.einsum("bhqd,bhkd->bhqk", q, k) * (Dh ** -0.5)
        idx = jnp.arange(S)
        mask = (idx[:, None] - idx[None, :] >= 0) & (idx[:, None] - idx[None, :] < W)
        scores = jnp.where(mask[None, None], scores, -1e9)
        p = _softmax(scores, axis=-1)
        o = jnp.einsum("bhqk,bhkd->bhqd", p, v)
        return (lambda x, *d: x.transpose(*d))(o, 0, 2, 1, 3).reshape(B, S, D) @ wo

    def _B_ref(u, A_re, A_im, B_re, B_im, C_re, C_im, log_dt, Dskip):
        Bsz, L, D = u.shape
        dt = jnp.exp(log_dt)[:, None]
        A = A_re + 1j * A_im
        Bc = B_re + 1j * B_im
        Cc = C_re + 1j * C_im
        logdA = dt * A
        dB = dt * Bc
        l = (lambda x, dt: x.astype(dt))(jnp.arange(L), A_re.dtype)
        P = jnp.exp(logdA[:, :, None] * l[None, None, :])
        K = jnp.einsum("dn,dnl,dn->dl", Cc, P, dB).real
        L2 = 2 * L
        Kp = jnp.pad(K, ((0, 0), (0, L)))
        up = (lambda x, *d: x.transpose(*d))(u, 0, 2, 1)
        up = jnp.pad(up, ((0, 0), (0, 0), (0, L)))
        Kf = (lambda x, axes=(-2,-1): jnp.fft.rfft2(x.astype(jnp.float32), axes=axes))(Kp[:, None, :], axes=(-2, -1))
        Uf = (lambda x, axes=(-2,-1): jnp.fft.rfft2(x.astype(jnp.float32), axes=axes))(up[:, :, None, :], axes=(-2, -1))
        Yf = Uf * Kf[None, :, :, :]
        y = (lambda x, s, axes=(-2,-1): jnp.fft.irfft2(x, s=s, axes=axes).astype(jnp.bfloat16))(Yf, (1, L2), axes=(-2, -1))[:, :, 0, :L]
        y = (lambda x, *d: x.transpose(*d))(y, 0, 2, 1) + u * Dskip[None, None, :]
        return y

    a = _A_ref(A_x, A_wqkv, A_wo)
    b = _B_ref(B_u, B_A_re, B_A_im, B_B_re, B_B_im, B_C_re, B_C_im, B_log_dt, B_Dskip)
    return jnp.concatenate([a, b], axis=-1)
```

```python
import functools
import math

import jax
import jax.numpy as jnp
from jax import lax
from jax.experimental import pallas as pl
from jax.experimental.pallas import tpu as pltpu

f32 = jnp.float32
bf16 = jnp.bfloat16
u32 = jnp.uint32
i32 = jnp.int32

S = 2048
D = 512
W = 256
TQ = 64
KW = 320
N = 128
NB = 16
G = 4
LOG2E = 1.4426950408889634
NEG = -1e9
NT = (((1,), (1,)), ((), ()))
TN = (((0,), (0,)), ((), ()))


def _b2u(x):
    return pltpu.bitcast(x, u32)


def _u2b(x):
    return pltpu.bitcast(x, bf16)


def _cmul(a, b):
    ar, ai = a
    br, bi = b
    return ar * br - ai * bi, ar * bi + ai * br


def _csq(a):
    ar, ai = a
    return ar * ar - ai * ai, (ar + ar) * ai


def _sincos(th):
    n = jnp.round(th * 0.6366197723675814)
    r = ((th - n * 1.5703125) - n * 4.837512969970703e-04) - n * 7.549789948768648e-08
    r2 = r * r
    s = r + r * r2 * (-1.6666654611e-1 + r2 * (8.3321608736e-3 + r2 * (-1.9515295891e-4)))
    c = 1.0 + r2 * (-0.5 + r2 * (4.166664568298827e-2 + r2 * (-1.388731625493765e-3 + r2 * 2.443315711809948e-5)))
    q = n.astype(i32)
    swap = (q & 1) == 1
    ss = jnp.where(swap, c, s)
    cc = jnp.where(swap, s, c)
    ss = jnp.where((q & 2) == 2, -ss, ss)
    cc = jnp.where(((q + 1) & 2) == 2, -cc, cc)
    return ss, cc


def _acc_exp(x):
    n = jnp.round(x * 1.4426950408889634)
    r = (x - n * 0.693359375) - n * (-2.12194440e-4)
    p = 1.0 + r * (1.0 + r * (0.5 + r * (1.6666667163e-1 + r * (4.1666667908e-2 + r * (
        8.3333337680e-3 + r * (1.3888889225e-3 + r * 1.9841270114e-4))))))
    e = lax.bitcast_convert_type((n.astype(i32) + 127) << 23, f32)
    return p * e


def _kernel(x_ref, wqkv_ref, wo_ref, u_ref, are, aim, bre, bim, cre, cim, ldt, dsk, out_ref,
            q_s, k_s, vt_s, ot_s, bias_s, rbuf, sbuf0, mbuf0, sbuf1, mbuf1,
            psr, psi, rr, ri, xsr, xsn, x16r, kt0, kt1,
            fm_s, gm_s, fa_s, g_s, kfr, kfi, kfs, utr, utd, uts, uraw, zb):
    kk = lax.broadcasted_iota(i32, (KW, 128), 0)
    qq = lax.broadcasted_iota(i32, (KW, 128), 1) % TQ
    for v in range(4):
        bias_s[v] = jnp.where(kk <= qq + TQ * v, 0.0, NEG).astype(f32)
    bias_s[4] = jnp.where((kk > qq) & (kk <= qq + W), 0.0, NEG).astype(f32)

    def proj_body(t, carry):
        r0 = pl.multiple_of(t * 128, 128)
        h0 = pl.multiple_of(t * 64, 64)
        xt = x_ref[pl.ds(r0, 128), :]
        qk = jnp.dot(xt, wqkv_ref[:, 0:1024], preferred_element_type=f32)
        q_s[pl.ds(h0, 64), :] = _b2u((qk[:, :512] * (0.25 * LOG2E)).astype(bf16))
        k_s[pl.ds(h0, 64), :] = _b2u(qk[:, 512:].astype(bf16))
        vt = lax.dot_general(wqkv_ref[:, 1024:1536], xt, (((0,), (1,)), ((), ())), preferred_element_type=f32)
        vt_s[0, :, pl.ds(r0, 128)] = _b2u(vt.astype(bf16))
        rolled = _b2u(pltpu.roll(vt, 64, 1).astype(bf16))

        @pl.when(t > 0)
        def _():
            lane_v = lax.broadcasted_iota(i32, (256, 128), 1)
            prev = rbuf[(t + 1) % 2]
            vt_s[1, :, pl.ds(pl.multiple_of(r0 - 128, 128), 128)] = jnp.where(lane_v < 64, prev, rolled)
        rbuf[t % 2] = rolled
        return carry
    lax.fori_loop(0, S // 128, proj_body, 0)
    vt_s[1, :, pl.ds(S - 128, 128)] = rbuf[1]

    lane = lax.broadcasted_iota(i32, (TQ // 2, 128), 1)
    lane2 = lax.broadcasted_iota(i32, (16, 128), 1)
    sbufs = (sbuf0, sbuf1)
    mbufs = (mbuf0, mbuf1)

    def stage1(un, slot, idx):
        I = un // 16
        j = un % 16
        g8 = j // 4
        p4 = j % 4
        l0 = pl.multiple_of(g8 * 128, 128)
        me = (lane >= 32 * p4) & (lane < 32 * p4 + 16)
        mo = (lane >= 32 * p4 + 16) & (lane < 32 * p4 + 32)
        for half in range(2):
            i = 2 * I + half
            q0h = pl.multiple_of(i * 32, 32)
            wsh = pl.multiple_of(jnp.maximum(i * 32 - 128, 0), 32)
            v = jnp.minimum(i, 4)
            q8 = q_s[pl.ds(q0h, 32), pl.ds(l0, 128)]
            zero = jnp.zeros_like(q8)
            qm = _u2b(jnp.concatenate([jnp.where(me, q8, zero), jnp.where(mo, q8, zero)], axis=0))
            k8 = _u2b(k_s[pl.ds(wsh, KW // 2), pl.ds(l0, 128)])
            st = lax.dot_general(k8, qm, NT, preferred_element_type=f32)
            st = st + bias_s[v]
            sbufs[slot][2 * idx + half] = st
            mbufs[slot][2 * idx + half] = jnp.max(st, axis=0, keepdims=True)

    def stage2(un, slot, idx):
        I = un // 16
        j = un % 16
        vrow = pl.multiple_of(16 * j, 16)
        wsa = pl.multiple_of(jnp.maximum(I * 128 - W, 0), 128)
        outs = []
        for half in range(2):
            st = sbufs[slot][2 * idx + half]
            m = mbufs[slot][2 * idx + half]
            p = jnp.exp2(st - m)
            l = jnp.sum(p, axis=0, keepdims=True)
            if half == 0:
                vt = vt_s[0, pl.ds(vrow, 16), pl.ds(wsa, KW)]
            else:
                cp = jnp.where(I >= 2, 1, 0)
                vt = vt_s[cp, pl.ds(vrow, 16), pl.ds(wsa, KW)]
            o = jnp.dot(_u2b(vt), p.astype(bf16), preferred_element_type=f32)
            outs.append(o * (1.0 / l))
        oa, ob = outs
        even = jnp.where(lane2 < 64, oa[0:16], pltpu.roll(ob[0:16], 64, 1))
        odd = jnp.where(lane2 < 64, pltpu.roll(oa[16:32], 64, 1), ob[16:32])
        res = jnp.concatenate([even, odd], axis=0).astype(bf16)
        ot_s[pl.ds(vrow, 16), pl.ds(pl.multiple_of(I * 128, 128), 128)] = _b2u(res)

    NG = 256 // G

    def half_body(t, slot):
        for g in range(G):
            stage2(t * G + g, slot, g)
            stage1((t + 1) * G + g, 1 - slot, g)

    def attn_body(t2, carry):
        half_body(2 * t2, 0)
        half_body(2 * t2 + 1, 1)
        return carry
    for g in range(G):
        stage1(jnp.int32(g), 0, g)
    lax.fori_loop(0, NG // 2 - 1, attn_body, 0)
    half_body(jnp.int32(NG - 2), 0)
    for g in range(G):
        stage2(jnp.int32((NG - 1) * G + g), (NG - 1) % 2, g)

    out_ref[:, 0:D] = lax.dot_general(_u2b(ot_s[...]), wo_ref[...], TN, preferred_element_type=f32).astype(out_ref.dtype)

    r_i = lax.broadcasted_iota(i32, (128, 128), 0)
    t_i = lax.broadcasted_iota(i32, (128, 128), 1)
    fr = jnp.where(r_i < 64, 2 * r_i, 2 * (r_i - 64) + 1)
    th = (((2 * fr + 1) * t_i) & 511).astype(f32) * (math.pi / 256.0)
    fm = jnp.concatenate([jnp.cos(th), -jnp.sin(th)], axis=0)
    fm_s[...] = fm.astype(bf16)
    fr2 = jnp.where(t_i < 64, 2 * t_i, 2 * (t_i - 64) + 1)
    th2 = (((2 * fr2 + 1) * r_i) & 511).astype(f32) * (math.pi / 256.0)
    gm_s[...] = (jnp.concatenate([jnp.cos(th2), -jnp.sin(th2)], axis=1).astype(bf16).astype(f32) * (1.0 / 128.0)).astype(bf16)
    e0 = jnp.where((lax.broadcasted_iota(i32, (16, 128), 0) == 0) & (lax.broadcasted_iota(i32, (16, 128), 1) == 0), 1.0, 0.0)
    fa_s[0] = jnp.concatenate([fm, e0], axis=0).astype(bf16)
    g_s[0] = jnp.zeros((256, 128), f32)
    for si, i0 in ((1, 2), (2, 4), (3, 8)):
        lag = (128 * i0 + r_i).astype(f32)
        lr = lag.astype(bf16).astype(f32).astype(i32) - 128 * i0
        sel = jnp.where(lr == t_i, 1.0, 0.0)
        fp = jnp.dot(fm, sel, preferred_element_type=f32, precision=lax.Precision.HIGHEST)
        fa_s[si] = jnp.concatenate([fp, e0], axis=0).astype(bf16)
        seln = jnp.where(lr == 128, 1.0, 0.0)
        g_s[si] = jnp.dot(fm, seln, preferred_element_type=f32, precision=lax.Precision.HIGHEST).astype(bf16).astype(f32)

    CH = 64

    def seeds_body(t, carry):
        r0 = pl.multiple_of(t * CH, CH)
        sl = pl.ds(r0, CH)
        dt = _acc_exp(ldt[sl, :].astype(f32)).astype(bf16).astype(f32)
        zr = dt * are[sl, :].astype(f32)
        zi = dt * aim[sl, :].astype(f32)
        dB = (dt * bre[sl, :].astype(f32), dt * bim[sl, :].astype(f32))
        w = _cmul((cre[sl, :].astype(f32), cim[sl, :].astype(f32)), dB)

        def direct(l):
            mag = jnp.exp(zr * l)
            s_, c_ = _sincos(zi * l)
            return mag * c_, mag * s_
        one = (jnp.ones_like(zr), jnp.zeros_like(zr))
        P = {0: one, 1: direct(1.0)}
        P[2] = _csq(P[1]); P[3] = _cmul(P[2], P[1]); P[4] = _csq(P[2])
        P[5] = _cmul(P[4], P[1]); P[6] = _cmul(P[4], P[2]); P[7] = _cmul(P[4], P[3])
        for s_ in range(8):
            psr[pl.ds(r0 * 8 + s_, CH, stride=8), :] = P[s_][0]
            psi[pl.ds(r0 * 8 + s_, CH, stride=8), :] = P[s_][1]
        R = {0: one, 1: direct(8.0)}
        for k in range(2, 16):
            h = 1 << (k.bit_length() - 1)
            R[k] = _csq(R[h // 2]) if k == h else _cmul(R[h], R[k - h])
        for k in range(1, 16):
            rr[k - 1, sl, :] = R[k][0]
            ri[k - 1, sl, :] = R[k][1]
        Q = {1: direct(128.0)}
        Q[2] = _csq(Q[1]); Q[4] = _csq(Q[2]); Q[8] = _csq(Q[4])
        X = {0: w}
        for a in range(1, 16):
            h = 1 << (a.bit_length() - 1)
            X[a] = _cmul(X[a - h], Q[h])
        X[16] = _cmul(X[8], Q[8])
        for a in range(16):
            xsr[a // 8, pl.ds(r0 * 8 + a % 8, CH, stride=8), :] = X[a][0]
            xsn[a // 8, pl.ds(r0 * 8 + a % 8, CH, stride=8), :] = -X[a][1]
        x16r[sl, :] = X[16][0]
        return carry
    lax.fori_loop(0, D // CH, seeds_body, 0)

    UNR = 8

    def chan(d):
        r8 = pl.ds(pl.multiple_of(d * 8, 8), 8)
        vr = psr[r8, :]
        vi = psi[r8, :]
        ers, eis = [vr], [vi]
        for k in range(1, 16):
            r_r = jnp.broadcast_to(rr[k - 1, pl.ds(d, 1), :], (8, N))
            r_i_ = jnp.broadcast_to(ri[k - 1, pl.ds(d, 1), :], (8, N))
            er, ei = _cmul((r_r, r_i_), (vr, vi))
            ers.append(er); eis.append(ei)
        et = jnp.concatenate([jnp.concatenate(ers, axis=0), jnp.concatenate(eis, axis=0)], axis=1).astype(bf16)
        xr = jnp.concatenate([xsr[0, r8, :], xsr[1, r8, :]], axis=0)
        xn = jnp.concatenate([xsn[0, r8, :], xsn[1, r8, :]], axis=0)
        x = jnp.concatenate([xr, xn], axis=1).astype(bf16)
        o = lax.dot_general(x, et, NT, preferred_element_type=f32)
        kt0[r8, :] = o[0:8]
        kt1[r8, :] = o[8:16]

    def chan_body(t, carry):
        for uu in range(UNR):
            chan(t * UNR + uu)
        return carry
    lax.fori_loop(0, D // UNR, chan_body, 0)

    ones8 = jnp.ones((8, 128), bf16)
    nf0 = lax.dot_general(ones8, x16r[...].astype(bf16), NT, preferred_element_type=f32)

    def kf_body(tt, nf):
        i = 15 - tt
        si = jnp.where(i < 2, 0, jnp.where(i < 4, 1, jnp.where(i < 8, 2, 3)))
        kt = lax.cond(i < 8, lambda: kt0[pl.ds(i & 7, D, stride=8), :], lambda: kt1[pl.ds(i & 7, D, stride=8), :])
        R = lax.dot_general(fa_s[si], kt.astype(bf16), NT, preferred_element_type=f32)
        g_ = g_s[si]
        kf = R[0:256] + jnp.concatenate([g_, g_, g_, g_], axis=1) * nf[0:1, :]
        kfr[i] = kf[0:128]; kfi[i] = kf[128:256]; kfs[i] = kf[0:128] + kf[128:256]
        return jnp.broadcast_to(R[256:257, :], (8, D))
    lax.fori_loop(0, NB, kf_body, nf0)

    uraw[...] = jnp.zeros_like(uraw)

    def uf_body(m, carry):
        um = u_ref[pl.ds(pl.multiple_of(m * 128, 128), 128), :]
        U = jnp.dot(fm_s[...], um, preferred_element_type=f32)
        Pv = uraw[...]
        ur, ui = U[0:128], U[128:256]
        pr, pi_ = Pv[0:128], Pv[128:256]
        tr = jnp.concatenate([ur[0:64] - pi_[0:64], ur[64:128] + pi_[64:128]], axis=0)
        ti = jnp.concatenate([ui[0:64] + pr[0:64], ui[64:128] - pr[64:128]], axis=0)
        utr[m] = tr; utd[m] = ti - tr; uts[m] = tr + ti
        uraw[...] = U
        return carry
    lax.fori_loop(0, NB, uf_body, 0)

    def pr_body(p, carry):
        g_ = p // 4
        cc = p % 4
        rs = pl.ds(pl.multiple_of(g_ * 8, 8), 8)
        ls = pl.ds(pl.multiple_of(cc * 128, 128), 128)
        K = [(kfr[i, rs, ls], kfi[i, rs, ls], kfs[i, rs, ls]) for i in range(NB)]
        U = [(utr[m, rs, ls], utd[m, rs, ls], uts[m, rs, ls]) for m in range(NB)]
        for j in range(NB):
            a1 = a2 = a3 = None
            for i in range(j + 1):
                kr, ki, ks = K[i]
                ur, ud, us = U[j - i]
                t1 = ur * ks; t2 = kr * ud; t3 = ki * us
                a1 = t1 if a1 is None else a1 + t1
                a2 = t2 if a2 is None else a2 + t2
                a3 = t3 if a3 is None else a3 + t3
            zb[j, rs, ls] = a1 - a3
            zb[j, pl.ds(pl.multiple_of(128 + g_ * 8, 8), 8), ls] = a1 + a2
        return carry
    lax.fori_loop(0, 64, pr_body, 0)

    def inv_body(j, carry):
        z = zb[j].astype(bf16)
        y = jnp.dot(gm_s[...], z, preferred_element_type=f32)
        rs = pl.ds(pl.multiple_of(j * 128, 128), 128)
        out_ref[rs, D:2 * D] = (y + u_ref[rs, :].astype(f32) * dsk[...].astype(f32)).astype(out_ref.dtype)
        return carry
    lax.fori_loop(0, NB, inv_body, 0)


@jax.jit
def pallas_concat_heads__sliding_block__ssm_conv_s4__prompt_kernel(
    A_x: jax.Array,
    A_wqkv: jax.Array,
    A_wo: jax.Array,
    B_u: jax.Array,
    B_A_re: jax.Array,
    B_A_im: jax.Array,
    B_B_re: jax.Array,
    B_B_im: jax.Array,
    B_C_re: jax.Array,
    B_C_im: jax.Array,
    B_log_dt: jax.Array,
    B_Dskip: jax.Array,
):
    out = pl.pallas_call(
        _kernel,
        out_shape=jax.ShapeDtypeStruct((S, 2 * D), bf16),
        scratch_shapes=[
            pltpu.VMEM((S // 2, D), u32),
            pltpu.VMEM((S // 2, D), u32),
            pltpu.VMEM((2, D // 2, S), u32),
            pltpu.VMEM((D // 2, S), u32),
            pltpu.VMEM((5, KW, 128), f32),
            pltpu.VMEM((2, D // 2, 128), u32),
            pltpu.VMEM((2 * G, KW, 128), f32), pltpu.VMEM((2 * G, 1, 128), f32),
            pltpu.VMEM((2 * G, KW, 128), f32), pltpu.VMEM((2 * G, 1, 128), f32),
            pltpu.VMEM((D * 8, N), f32), pltpu.VMEM((D * 8, N), f32),
            pltpu.VMEM((15, D, N), f32), pltpu.VMEM((15, D, N), f32),
            pltpu.VMEM((2, D * 8, N), f32), pltpu.VMEM((2, D * 8, N), f32),
            pltpu.VMEM((D, N), f32),
            pltpu.VMEM((D * 8, 128), f32), pltpu.VMEM((D * 8, 128), f32),
            pltpu.VMEM((256, 128), bf16), pltpu.VMEM((128, 256), bf16),
            pltpu.VMEM((4, 272, 128), bf16), pltpu.VMEM((4, 256, 128), f32),
            pltpu.VMEM((NB, 128, D), f32), pltpu.VMEM((NB, 128, D), f32), pltpu.VMEM((NB, 128, D), f32),
            pltpu.VMEM((NB, 128, D), f32), pltpu.VMEM((NB, 128, D), f32), pltpu.VMEM((NB, 128, D), f32),
            pltpu.VMEM((256, D), f32),
            pltpu.VMEM((NB, 256, D), f32),
        ],
        compiler_params=pltpu.CompilerParams(vmem_limit_bytes=120 * 1024 * 1024),
    )(
        A_x.reshape(S, D), A_wqkv, A_wo, B_u.reshape(S, D),
        B_A_re, B_A_im, B_B_re, B_B_im, B_C_re, B_C_im,
        B_log_dt.reshape(D, 1), B_Dskip.reshape(1, D),
    )
    return out.reshape(1, S, 2 * D)
```

```python
import functools
import math

import jax
import jax.numpy as jnp
from jax import lax
from jax.experimental import pallas as pl
from jax.experimental.pallas import tpu as pltpu

f32 = jnp.float32
bf16 = jnp.bfloat16
u32 = jnp.uint32
i32 = jnp.int32

S = 2048
D = 512
W = 256
TQ = 64
KW = 320
N = 128
NB = 16
G = 4
CH = 32
LOG2E = 1.4426950408889634
NEG = -1e9
NT = (((1,), (1,)), ((), ()))
TN = (((0,), (0,)), ((), ()))


def _b2u(x):
    return pltpu.bitcast(x, u32)


def _u2b(x):
    return pltpu.bitcast(x, bf16)


def _mo(x, m):
    return x if isinstance(x, int) else pl.multiple_of(x, m)


def _cmul(a, b):
    ar, ai = a
    br, bi = b
    return ar * br - ai * bi, ar * bi + ai * br


def _csq(a):
    ar, ai = a
    return ar * ar - ai * ai, (ar + ar) * ai


def _sincos(th):
    n = jnp.round(th * 0.6366197723675814)
    r = ((th - n * 1.5703125) - n * 4.837512969970703e-04) - n * 7.549789948768648e-08
    r2 = r * r
    s = r + r * r2 * (-1.6666654611e-1 + r2 * (8.3321608736e-3 + r2 * (-1.9515295891e-4)))
    c = 1.0 + r2 * (-0.5 + r2 * (4.166664568298827e-2 + r2 * (-1.388731625493765e-3 + r2 * 2.443315711809948e-5)))
    q = n.astype(i32)
    swap = (q & 1) == 1
    ss = jnp.where(swap, c, s)
    cc = jnp.where(swap, s, c)
    ss = jnp.where((q & 2) == 2, -ss, ss)
    cc = jnp.where(((q + 1) & 2) == 2, -cc, cc)
    return ss, cc


def _acc_exp(x):
    n = jnp.round(x * 1.4426950408889634)
    r = (x - n * 0.693359375) - n * (-2.12194440e-4)
    p = 1.0 + r * (1.0 + r * (0.5 + r * (1.6666667163e-1 + r * (4.1666667908e-2 + r * (
        8.3333337680e-3 + r * (1.3888889225e-3 + r * 1.9841270114e-4))))))
    e = lax.bitcast_convert_type((n.astype(i32) + 127) << 23, f32)
    return p * e


def _interleave(*gens, weights=None):
    gens = list(gens)
    alive = [True] * len(gens)
    while any(alive):
        for k, g in enumerate(gens):
            if not alive[k]:
                continue
            for _ in range(1 if weights is None else weights[k]):
                try:
                    next(g)
                except StopIteration:
                    alive[k] = False
                    break


def _kernel(x_h, wqkv_h, wo_h, u_h, are_h, aim_h, bre_h, bim_h, cre_h, cim_h, ldt_h, dsk_h, out_h,
            x_ref, wqkv_ref, wo_ref, u_ref, are, aim, bre, bim, cre, cim, ldt, dsk, out_ref, dsem, osem,
            q_s, k_s, vt_s, ot_s, bias_s, rbuf, sbuf0, mbuf0, sbuf1, mbuf1, wvt_s,
            psr, psi, rr, ri, xsr, xsn, x16r, kt,
            fm_s, gm_s, fa_s, g_s, kfr, kfi, kfs, utr, utd, uts, uraw, zb, zbuf, tsem, *, cfg):
    zv = jnp.full((8, 128), pl.semaphore_read(tsem), i32).astype(u32)
    srcs = [wqkv_h, x_h, ldt_h, are_h, aim_h, bre_h, bim_h, cre_h, cim_h, u_h, dsk_h, wo_h]
    dsts = [wqkv_ref, x_ref, ldt, are, aim, bre, bim, cre, cim, u_ref, dsk, wo_ref]
    cps = [pltpu.make_async_copy(a, b, dsem.at[k]) for k, (a, b) in enumerate(zip(srcs, dsts))]
    for cp in cps:
        cp.start()
    kk = lax.broadcasted_iota(i32, (KW, 128), 0)
    qq = lax.broadcasted_iota(i32, (KW, 128), 1) % TQ
    for v in range(4):
        bias_s[v] = jnp.where(kk <= qq + TQ * v, 0.0, NEG).astype(f32)
    bias_s[4] = jnp.where((kk > qq) & (kk <= qq + W), 0.0, NEG).astype(f32)

    r_i = lax.broadcasted_iota(i32, (128, 128), 0)
    t_i = lax.broadcasted_iota(i32, (128, 128), 1)
    fr = jnp.where(r_i < 64, 2 * r_i, 2 * (r_i - 64) + 1)
    th = (((2 * fr + 1) * t_i) & 511).astype(f32) * (math.pi / 256.0)
    fm = jnp.concatenate([jnp.cos(th), -jnp.sin(th)], axis=0)
    fm_s[...] = fm.astype(bf16)
    fr2 = jnp.where(t_i < 64, 2 * t_i, 2 * (t_i - 64) + 1)
    th2 = (((2 * fr2 + 1) * r_i) & 511).astype(f32) * (math.pi / 256.0)
    gm_s[...] = (jnp.concatenate([jnp.cos(th2), -jnp.sin(th2)], axis=1).astype(bf16).astype(f32) * (1.0 / 128.0)).astype(bf16)
    e0 = jnp.where((lax.broadcasted_iota(i32, (16, 128), 0) == 0) & (lax.broadcasted_iota(i32, (16, 128), 1) == 0), 1.0, 0.0)
    fa_s[0] = jnp.concatenate([fm, e0], axis=0).astype(bf16)
    g_s[0] = jnp.zeros((256, 128), f32)
    for si, i0 in ((1, 2), (2, 4), (3, 8)):
        lag = (128 * i0 + r_i).astype(f32)
        lr = lag.astype(bf16).astype(f32).astype(i32) - 128 * i0
        sel = jnp.where(lr == t_i, 1.0, 0.0)
        fp = jnp.dot(fm, sel, preferred_element_type=f32, precision=lax.Precision.HIGHEST)
        fa_s[si] = jnp.concatenate([fp, e0], axis=0).astype(bf16)
        seln = jnp.where(lr == 128, 1.0, 0.0)
        g_s[si] = jnp.dot(fm, seln, preferred_element_type=f32, precision=lax.Precision.HIGHEST).astype(bf16).astype(f32)

    for cp in cps[:-1]:
        cp.wait()
    wvt_s[...] = _b2u(wqkv_ref[:, 1024:1536].astype(f32).T.astype(bf16))
    rbuf[1] = jnp.zeros((D // 2, 128), u32)
    uraw[...] = jnp.zeros_like(uraw)

    dep = {}

    def tokdep(w):
        if "tok" not in dep or not cfg.get("tok", 0):
            return w
        tok = lax.bitcast_convert_type(dep.pop("tok"), u32)[0:8, 0:128] & zv
        top = _u2b(_b2u(w[0:16, 0:128]) | tok)
        if w.shape[1] > 128:
            top = jnp.concatenate([top, w[0:16, 128:]], axis=1)
        return jnp.concatenate([top, w[16:]], axis=0)

    def adep(v):
        lag = cfg.get("lag", 0)
        h = dep.get("ahist", [])
        if not lag or len(h) < lag:
            return v
        tk = lax.bitcast_convert_type(h[-lag], u32) & zv
        if v.shape[0] != 8:
            tk = jnp.concatenate([tk] * (v.shape[0] // 8), axis=0)
        return lax.bitcast_convert_type(lax.bitcast_convert_type(v, u32) | tk[:, 0:v.shape[1]], f32)

    def seeds_small(c, CHS):
        r0 = _mo(c * CHS, CHS)
        sl = pl.ds(r0, CHS)

        def st_p(s_, val):
            psr[pl.ds(r0 * 8 + s_, CHS, stride=8), :] = val[0]
            psi[pl.ds(r0 * 8 + s_, CHS, stride=8), :] = val[1]

        def st_x(a, val):
            xsr[a // 8, pl.ds(r0 * 8 + a % 8, CHS, stride=8), :] = val[0]
            xsn[a // 8, pl.ds(r0 * 8 + a % 8, CHS, stride=8), :] = -val[1]

        def start():
            dt = adep(_acc_exp(ldt[sl, :].astype(f32)).astype(bf16).astype(f32))
            zr = dt * are[sl, :].astype(f32)
            zi = dt * aim[sl, :].astype(f32)

            def direct(l):
                mag = jnp.exp(zr * l)
                s_, c_ = _sincos(zi * l)
                return mag * c_, mag * s_
            return dt, direct
        dt, direct = start()
        one = (jnp.ones((CHS, N), f32), jnp.zeros((CHS, N), f32))
        st_p(0, one)
        p1 = direct(1.0); st_p(1, p1)
        p2 = _csq(p1); st_p(2, p2)
        p3 = _cmul(p2, p1); st_p(3, p3)
        p4 = _csq(p2); st_p(4, p4)
        st_p(5, _cmul(p4, p1)); st_p(6, _cmul(p4, p2)); p7 = _cmul(p4, p3); st_p(7, p7)
        dep["tok"] = p7[0]
        yield
        dt, direct = start()
        R = {1: direct(8.0)}
        rr[0, sl, :] = R[1][0]; ri[0, sl, :] = R[1][1]
        for k in range(2, 16):
            h = 1 << (k.bit_length() - 1)
            R[k] = _csq(R[h // 2]) if k == h else _cmul(R[h], R[k - h])
            rr[k - 1, sl, :] = R[k][0]; ri[k - 1, sl, :] = R[k][1]
        dep["tok"] = R[15][0]
        yield
        dt, direct = start()
        dB = (dt * bre[sl, :].astype(f32), dt * bim[sl, :].astype(f32))
        w = _cmul((cre[sl, :].astype(f32), cim[sl, :].astype(f32)), dB)
        Q = {1: direct(128.0)}
        Q[2] = _csq(Q[1]); Q[4] = _csq(Q[2]); Q[8] = _csq(Q[4])
        X = {0: w}
        st_x(0, w)
        for a in range(1, 16):
            h = 1 << (a.bit_length() - 1)
            X[a] = _cmul(X[a - h], Q[h])
            st_x(a, X[a])
        x16v = _cmul(X[8], Q[8])[0]
        x16r[sl, :] = x16v
        dep["tok"] = x16v
        yield

    def seeds_gen(t):
        CHS = cfg.get("chs", 32)
        nsub = CH // CHS
        for sub in range(nsub):
            yield from seeds_small(t * nsub + sub, CHS)

    def chan(d):
        r8 = pl.ds(_mo(d * 8, 8), 8)
        vr = psr[r8, :]
        vi = psi[r8, :]
        ers, eis = [vr], [vi]
        for k in range(1, 16):
            if cfg.get("s0", 0):
                r_r = rr[k - 1, pl.ds(d, 8, stride=0), :]
                r_i_ = ri[k - 1, pl.ds(d, 8, stride=0), :]
            else:
                r_r = jnp.broadcast_to(rr[k - 1, pl.ds(d, 1), :], (8, N))
                r_i_ = jnp.broadcast_to(ri[k - 1, pl.ds(d, 1), :], (8, N))
            er, ei = _cmul((r_r, r_i_), (vr, vi))
            ers.append(er); eis.append(ei)
        et = jnp.concatenate([jnp.concatenate(ers, axis=0), jnp.concatenate(eis, axis=0)], axis=1).astype(bf16)
        xr = jnp.concatenate([xsr[0, r8, :], xsr[1, r8, :]], axis=0)
        xn = jnp.concatenate([xsn[0, r8, :], xsn[1, r8, :]], axis=0)
        x = jnp.concatenate([xr, xn], axis=1).astype(bf16)
        o = lax.dot_general(x, et, NT, preferred_element_type=f32)
        kt[0, r8, :] = o[0:8]
        kt[1, r8, :] = o[8:16]

    def chan_gen(d0, n):
        for k in range(n):
            chan(d0 + k)
            yield

    def uf_gen(m):
        um = u_ref[pl.ds(_mo(m * 128, 128), 128), :]
        U = jnp.dot(fm_s[...], um, preferred_element_type=f32)
        yield
        Pv = uraw[...]
        ur, ui = U[0:128], U[128:256]
        pr, pi_ = Pv[0:128], Pv[128:256]
        tr = jnp.concatenate([ur[0:64] - pi_[0:64], ur[64:128] + pi_[64:128]], axis=0)
        ti = jnp.concatenate([ui[0:64] + pr[0:64], ui[64:128] - pr[64:128]], axis=0)
        utr[m] = tr; utd[m] = ti - tr; uts[m] = tr + ti
        uraw[...] = U
        yield

    lane_v = lax.broadcasted_iota(i32, (256, 128), 1)

    def proj_gen(t):
        r0 = _mo(t * 128, 128)
        h0 = _mo(t * 64, 64)
        xt = x_ref[pl.ds(r0, 128), :]
        for nb in range(8):
            qk = jnp.dot(xt, tokdep(wqkv_ref[:, 128 * nb:128 * nb + 128]), preferred_element_type=f32)
            dep.setdefault("ahist", []).append(qk[0:8])
            if nb < 4:
                q_s[pl.ds(h0, 64), 128 * nb:128 * nb + 128] = _b2u((qk * (0.25 * LOG2E)).astype(bf16))
            else:
                k_s[pl.ds(h0, 64), 128 * (nb - 4):128 * (nb - 4) + 128] = _b2u(qk.astype(bf16))
            yield
        for rb in range(4):
            vt = lax.dot_general(tokdep(_u2b(wvt_s[64 * rb:64 * rb + 64, :])), xt, NT, preferred_element_type=f32)
            dep.setdefault("ahist", []).append(vt[0:8])
            vt_s[0, 64 * rb:64 * rb + 64, pl.ds(r0, 128)] = _b2u(vt.astype(bf16))
            rolled = _b2u(pltpu.roll(vt, 64, 1).astype(bf16))
            if cfg.get("dep", 0) and rb == 3 and "tok" in dep:
                tok = lax.bitcast_convert_type(dep["tok"], u32)
                zer = rbuf[2 + 0 * 0, 0:tok.shape[0], :] if False else zbuf[...]
                rolled = rolled | jnp.concatenate([tok[0:8] & zer, ] * 8, axis=0)
            lane_ = lax.broadcasted_iota(i32, (64, 128), 1)
            if isinstance(t, int):
                pc = max(r0 - 128, 0)
            else:
                pc = pl.multiple_of(jnp.maximum(r0 - 128, 0), 128)
            prev = rbuf[(t + 1) % 2, 64 * rb:64 * rb + 64, :]
            vt_s[1, 64 * rb:64 * rb + 64, pl.ds(pc, 128)] = jnp.where(lane_ < 64, prev, rolled)
            rbuf[t % 2, 64 * rb:64 * rb + 64, :] = rolled
            yield

    mode = cfg.get("l1", "seq")

    def proj_iter(t):
        dep.clear()
        if mode == "seq":
            _interleave(proj_gen(t)); _interleave(seeds_gen(t)); _interleave(uf_gen(t))
        else:
            _interleave(seeds_gen(t), proj_gen(t), uf_gen(t))

    def proj_body(t, carry):
        proj_iter(t)
        return carry
    if cfg.get("n1", 16):
        lax.fori_loop(0, cfg.get("n1", 16), proj_body, 0)
    vt_s[1, :, pl.ds(S - 128, 128)] = rbuf[1]

    lane = lax.broadcasted_iota(i32, (TQ // 2, 128), 1)
    lane2 = lax.broadcasted_iota(i32, (16, 128), 1)
    sbufs = (sbuf0, sbuf1)
    mbufs = (mbuf0, mbuf1)

    def stage1(un, slot, idx):
        I = un // 16
        j = un % 16
        g8 = j // 4
        p4 = j % 4
        l0 = _mo(g8 * 128, 128)
        me = (lane >= 32 * p4) & (lane < 32 * p4 + 16)
        mo = (lane >= 32 * p4 + 16) & (lane < 32 * p4 + 32)
        for half in range(2):
            i = 2 * I + half
            q0h = _mo(i * 32, 32)
            if isinstance(i, int):
                wsh = max(i * 32 - 128, 0); v = min(i, 4)
            else:
                wsh = pl.multiple_of(jnp.maximum(i * 32 - 128, 0), 32); v = jnp.minimum(i, 4)
            q8 = q_s[pl.ds(q0h, 32), pl.ds(l0, 128)]
            zero = jnp.zeros_like(q8)
            qm = _u2b(jnp.concatenate([jnp.where(me, q8, zero), jnp.where(mo, q8, zero)], axis=0))
            k8 = _u2b(k_s[pl.ds(wsh, KW // 2), pl.ds(l0, 128)])
            st = lax.dot_general(k8, qm, NT, preferred_element_type=f32)
            st = st + bias_s[v]
            sbufs[slot][2 * idx + half] = st
            mbufs[slot][2 * idx + half] = jnp.max(st, axis=0, keepdims=True)

    def stage2(un, slot, idx):
        I = un // 16
        j = un % 16
        vrow = _mo(16 * j, 16)
        if isinstance(I, int):
            wsa = max(I * 128 - W, 0); cp = 1 if I >= 2 else 0
        else:
            wsa = pl.multiple_of(jnp.maximum(I * 128 - W, 0), 128); cp = jnp.where(I >= 2, 1, 0)
        outs = []
        for half in range(2):
            st = sbufs[slot][2 * idx + half]
            m = mbufs[slot][2 * idx + half]
            p = jnp.exp2(st - m)
            l = jnp.sum(p, axis=0, keepdims=True)
            vt = vt_s[0 if half == 0 else cp, pl.ds(vrow, 16), pl.ds(wsa, KW)]
            o = jnp.dot(_u2b(vt), p.astype(bf16), preferred_element_type=f32)
            outs.append(o * (1.0 / l))
        oa, ob = outs
        even = jnp.where(lane2 < 64, oa[0:16], pltpu.roll(ob[0:16], 64, 1))
        odd = jnp.where(lane2 < 64, pltpu.roll(oa[16:32], 64, 1), ob[16:32])
        res = jnp.concatenate([even, odd], axis=0).astype(bf16)
        ot_s[pl.ds(vrow, 16), pl.ds(_mo(I * 128, 128), 128)] = _b2u(res)

    NG = 256 // G

    def half_body(t, slot):
        for g in range(G):
            stage2(t * G + g, slot, g)
            chan(t * 8 + 2 * g)
            stage1((t + 1) * G + g, 1 - slot, g)
            chan(t * 8 + 2 * g + 1)

    def attn_body(t2, carry):
        half_body(2 * t2, 0)
        half_body(2 * t2 + 1, 1)
        return carry
    if not cfg.get("n2", 1):
        def cb(t, c):
            for uu in range(8):
                chan(t * 8 + uu)
            return c
        lax.fori_loop(0, 64, cb, 0)
        ot_s[...] = _b2u(_u2b(q_s[...]).T[:512, :]) if False else ot_s[...]
        ot_s[:, 0:512] = k_s[0:256, :] + vt_s[1, :, 0:512] + vt_s[0, :, 0:512]
        ot_s[:, 512:2048] = jnp.zeros((256, 1536), u32) + q_s[0:256, 0:1]
    if cfg.get("n2", 1):
        for g in range(G):
            stage1(g, 0, g)
        lax.fori_loop(0, NG // 2 - 1, attn_body, 0)
        half_body(NG - 2, 0)
        for g in range(G):
            stage2((NG - 1) * G + g, (NG - 1) % 2, g)
            chan((NG - 1) * 8 + 2 * g)
            chan((NG - 1) * 8 + 2 * g + 1)

    if not cfg.get("n3", 1):
        out_ref[...] = jnp.zeros_like(out_ref)
        cps[-1].wait()
        oc = pltpu.make_async_copy(out_ref, out_h, osem.at[0]); oc.start(); oc.wait()
        return

    cps[-1].wait()
    out_ref[:, 0:D] = lax.dot_general(_u2b(ot_s[...]), wo_ref[...], TN, preferred_element_type=f32).astype(out_ref.dtype)
    ocpA = pltpu.make_async_copy(out_ref.at[:, 0:D], out_h.at[:, 0:D], osem.at[NB])
    ocpA.start()

    ones8 = jnp.ones((8, 128), bf16)
    nf0 = lax.dot_general(ones8, x16r[...].astype(bf16), NT, preferred_element_type=f32)

    def kf_body(tt, nf):
        i = 15 - tt
        si = jnp.where(i < 2, 0, jnp.where(i < 4, 1, jnp.where(i < 8, 2, 3)))
        ktv = kt[i >> 3, pl.ds(i & 7, D, stride=8), :]
        R = lax.dot_general(fa_s[si], ktv.astype(bf16), NT, preferred_element_type=f32)
        g_ = g_s[si]
        kf = R[0:256] + jnp.concatenate([g_, g_, g_, g_], axis=1) * nf[0:1, :]
        kfr[i] = kf[0:128]; kfi[i] = kf[128:256]; kfs[i] = kf[0:128] + kf[128:256]
        return jnp.broadcast_to(R[256:257, :], (8, D))
    lax.fori_loop(0, NB, kf_body, nf0)

    def pr_body(p, carry):
        g_ = p // 4
        cc = p % 4
        rs = pl.ds(pl.multiple_of(g_ * 8, 8), 8)
        ls = pl.ds(pl.multiple_of(cc * 128, 128), 128)
        K = [(kfr[i, rs, ls], kfi[i, rs, ls], kfs[i, rs, ls]) for i in range(NB)]
        U = [(utr[m, rs, ls], utd[m, rs, ls], uts[m, rs, ls]) for m in range(NB)]
        for j in range(NB):
            a1 = a2 = a3 = None
            for i in range(j + 1):
                kr, ki, ks = K[i]
                ur, ud, us = U[j - i]
                t1 = ur * ks; t2 = kr * ud; t3 = ki * us
                a1 = t1 if a1 is None else a1 + t1
                a2 = t2 if a2 is None else a2 + t2
                a3 = t3 if a3 is None else a3 + t3
            zb[j, rs, ls] = a1 - a3
            zb[j, pl.ds(pl.multiple_of(128 + g_ * 8, 8), 8), ls] = a1 + a2
        return carry
    lax.fori_loop(0, 64, pr_body, 0)

    def inv_body(j, carry):
        z = zb[j].astype(bf16)
        y = jnp.dot(gm_s[...], z, preferred_element_type=f32)
        rs = pl.ds(pl.multiple_of(j * 128, 128), 128)
        out_ref[rs, D:2 * D] = (y + u_ref[rs, :].astype(f32) * dsk[...].astype(f32)).astype(out_ref.dtype)
        pltpu.make_async_copy(out_ref.at[rs, D:2 * D], out_h.at[rs, D:2 * D], osem.at[j]).start()
        return carry
    lax.fori_loop(0, NB, inv_body, 0)
    for j in range(NB):
        pltpu.make_async_copy(out_ref.at[pl.ds(j * 128, 128), D:2 * D], out_h.at[pl.ds(j * 128, 128), D:2 * D], osem.at[j]).wait()
    ocpA.wait()


_CFG = {"l1": "seq", "s0": 1}


def build(cfg):
    @jax.jit
    def pallas_concat_heads__sliding_block__ssm_conv_s4__prompt_kernel(
        A_x, A_wqkv, A_wo, B_u, B_A_re, B_A_im, B_B_re, B_B_im, B_C_re, B_C_im, B_log_dt, B_Dskip,
    ):
        out = pl.pallas_call(
            functools.partial(_kernel, cfg=cfg),
            out_shape=jax.ShapeDtypeStruct((S, 2 * D), bf16),
            in_specs=[pl.BlockSpec(memory_space=pl.ANY)] * 12,
            out_specs=pl.BlockSpec(memory_space=pl.ANY),
            scratch_shapes=[
                pltpu.VMEM((S, D), bf16), pltpu.VMEM((D, 3 * D), bf16), pltpu.VMEM((D, D), bf16), pltpu.VMEM((S, D), bf16),
                pltpu.VMEM((D, N), bf16), pltpu.VMEM((D, N), bf16), pltpu.VMEM((D, N), bf16),
                pltpu.VMEM((D, N), bf16), pltpu.VMEM((D, N), bf16), pltpu.VMEM((D, N), bf16),
                pltpu.VMEM((D, 1), bf16), pltpu.VMEM((1, D), bf16), pltpu.VMEM((S, 2 * D), bf16),
                pltpu.SemaphoreType.DMA((12,)), pltpu.SemaphoreType.DMA((NB + 1,)),
                pltpu.VMEM((S // 2, D), u32),
                pltpu.VMEM((S // 2, D), u32),
                pltpu.VMEM((2, D // 2, S), u32),
                pltpu.VMEM((D // 2, S), u32),
                pltpu.VMEM((5, KW, 128), f32),
                pltpu.VMEM((2, D // 2, 128), u32),
                pltpu.VMEM((2 * G, KW, 128), f32), pltpu.VMEM((2 * G, 1, 128), f32),
                pltpu.VMEM((2 * G, KW, 128), f32), pltpu.VMEM((2 * G, 1, 128), f32),
                pltpu.VMEM((D // 2, D), u32),
                pltpu.VMEM((D * 8, N), f32), pltpu.VMEM((D * 8, N), f32),
                pltpu.VMEM((15, D, N), f32), pltpu.VMEM((15, D, N), f32),
                pltpu.VMEM((2, D * 8, N), f32), pltpu.VMEM((2, D * 8, N), f32),
                pltpu.VMEM((D, N), f32),
                pltpu.VMEM((2, D * 8, 128), f32),
                pltpu.VMEM((256, 128), bf16), pltpu.VMEM((128, 256), bf16),
                pltpu.VMEM((4, 272, 128), bf16), pltpu.VMEM((4, 256, 128), f32),
                pltpu.VMEM((NB, 128, D), f32), pltpu.VMEM((NB, 128, D), f32), pltpu.VMEM((NB, 128, D), f32),
                pltpu.VMEM((NB, 128, D), f32), pltpu.VMEM((NB, 128, D), f32), pltpu.VMEM((NB, 128, D), f32),
                pltpu.VMEM((256, D), f32),
                pltpu.VMEM((NB, 256, D), f32),
                pltpu.VMEM((8, 128), u32),
                pltpu.SemaphoreType.REGULAR,
            ],
            compiler_params=pltpu.CompilerParams(vmem_limit_bytes=120 * 1024 * 1024),
        )(
            A_x.reshape(S, D), A_wqkv, A_wo, B_u.reshape(S, D),
            B_A_re, B_A_im, B_B_re, B_B_im, B_C_re, B_C_im,
            B_log_dt.reshape(D, 1), B_Dskip.reshape(1, D),
        )
        return out.reshape(1, S, 2 * D)
    return pallas_concat_heads__sliding_block__ssm_conv_s4__prompt_kernel


pallas_concat_heads__sliding_block__ssm_conv_s4__prompt_kernel = build(_CFG)
```

```python
import functools
import math

import jax
import jax.numpy as jnp
from jax import lax
from jax.experimental import pallas as pl
from jax.experimental.pallas import tpu as pltpu

f32 = jnp.float32
bf16 = jnp.bfloat16
u32 = jnp.uint32
i32 = jnp.int32

S = 2048
D = 512
W = 256
TQ = 64
KW = 320
N = 128
NB = 16
G = 8
CH = 32
LOG2E = 1.4426950408889634
NEG = -1e9
NT = (((1,), (1,)), ((), ()))
TN = (((0,), (0,)), ((), ()))


def _b2u(x):
    return pltpu.bitcast(x, u32)


def _u2b(x):
    return pltpu.bitcast(x, bf16)


def _mo(x, m):
    return x if isinstance(x, int) else pl.multiple_of(x, m)


def _cmul(a, b):
    ar, ai = a
    br, bi = b
    return ar * br - ai * bi, ar * bi + ai * br


def _csq(a):
    ar, ai = a
    return ar * ar - ai * ai, (ar + ar) * ai


def _sincos(th):
    n = jnp.round(th * 0.6366197723675814)
    r = ((th - n * 1.5703125) - n * 4.837512969970703e-04) - n * 7.549789948768648e-08
    r2 = r * r
    s = r + r * r2 * (-1.6666654611e-1 + r2 * (8.3321608736e-3 + r2 * (-1.9515295891e-4)))
    c = 1.0 + r2 * (-0.5 + r2 * (4.166664568298827e-2 + r2 * (-1.388731625493765e-3 + r2 * 2.443315711809948e-5)))
    q = n.astype(i32)
    swap = (q & 1) == 1
    ss = jnp.where(swap, c, s)
    cc = jnp.where(swap, s, c)
    ss = jnp.where((q & 2) == 2, -ss, ss)
    cc = jnp.where(((q + 1) & 2) == 2, -cc, cc)
    return ss, cc


def _acc_exp(x):
    n = jnp.round(x * 1.4426950408889634)
    r = (x - n * 0.693359375) - n * (-2.12194440e-4)
    p = 1.0 + r * (1.0 + r * (0.5 + r * (1.6666667163e-1 + r * (4.1666667908e-2 + r * (
        8.3333337680e-3 + r * (1.3888889225e-3 + r * 1.9841270114e-4))))))
    e = lax.bitcast_convert_type((n.astype(i32) + 127) << 23, f32)
    return p * e


def _interleave(*gens, weights=None):
    gens = list(gens)
    alive = [True] * len(gens)
    while any(alive):
        for k, g in enumerate(gens):
            if not alive[k]:
                continue
            for _ in range(1 if weights is None else weights[k]):
                try:
                    next(g)
                except StopIteration:
                    alive[k] = False
                    break


def _kernel(x_h, wqkv_h, wo_h, u_h, are_h, aim_h, bre_h, bim_h, cre_h, cim_h, ldt_h, dsk_h, out_h,
            x_ref, wqkv_ref, wo_ref, u_ref, are, aim, bre, bim, cre, cim, ldt, dsk, out_ref, dsem, osem,
            q_s, k_s, vt_s, ot_s, bias_s, rbuf, sbuf0, mbuf0, sbuf1, mbuf1, wvt_s,
            psr, psi, rr, ri, xsr, xsn, x16r, kt,
            fm_s, gm_s, fa_s, g_s, kfr, kfi, kfs, utr, utd, uts, uraw, zb, zbuf, tsem, *, cfg):
    zv = jnp.full((8, 128), pl.semaphore_read(tsem), i32).astype(u32)
    srcs = [wqkv_h, ldt_h, are_h, aim_h, bre_h, bim_h, cre_h, cim_h, x_h.at[0:S // 2], x_h.at[S // 2:S], u_h, dsk_h, wo_h]
    dsts = [wqkv_ref, ldt, are, aim, bre, bim, cre, cim, x_ref.at[0:S // 2], x_ref.at[S // 2:S], u_ref, dsk, wo_ref]
    cps = [pltpu.make_async_copy(a, b, dsem.at[k]) for k, (a, b) in enumerate(zip(srcs, dsts))]
    for cp in cps:
        cp.start()
    kk = lax.broadcasted_iota(i32, (KW, 128), 0)
    qq = lax.broadcasted_iota(i32, (KW, 128), 1) % TQ
    for v in range(4):
        bias_s[v] = jnp.where(kk <= qq + TQ * v, 0.0, NEG).astype(f32)
    bias_s[4] = jnp.where((kk > qq) & (kk <= qq + W), 0.0, NEG).astype(f32)

    r_i = lax.broadcasted_iota(i32, (128, 128), 0)
    t_i = lax.broadcasted_iota(i32, (128, 128), 1)
    fr = jnp.where(r_i < 64, 2 * r_i, 2 * (r_i - 64) + 1)
    th = (((2 * fr + 1) * t_i) & 511).astype(f32) * (math.pi / 256.0)
    fm = jnp.concatenate([jnp.cos(th), -jnp.sin(th)], axis=0)
    fm_s[...] = fm.astype(bf16)
    fr2 = jnp.where(t_i < 64, 2 * t_i, 2 * (t_i - 64) + 1)
    th2 = (((2 * fr2 + 1) * r_i) & 511).astype(f32) * (math.pi / 256.0)
    gm_s[...] = (jnp.concatenate([jnp.cos(th2), -jnp.sin(th2)], axis=1).astype(bf16).astype(f32) * (1.0 / 128.0)).astype(bf16)
    e0 = jnp.where((lax.broadcasted_iota(i32, (16, 128), 0) == 0) & (lax.broadcasted_iota(i32, (16, 128), 1) == 0), 1.0, 0.0)
    fa_s[0] = jnp.concatenate([fm, e0], axis=0).astype(bf16)
    g_s[0] = jnp.zeros((256, 128), f32)
    for si, i0 in ((1, 2), (2, 4), (3, 8)):
        lag = (128 * i0 + r_i).astype(f32)
        lr = lag.astype(bf16).astype(f32).astype(i32) - 128 * i0
        sel = jnp.where(lr == t_i, 1.0, 0.0)
        fp = jnp.dot(fm, sel, preferred_element_type=f32, precision=lax.Precision.HIGHEST)
        fa_s[si] = jnp.concatenate([fp, e0], axis=0).astype(bf16)
        seln = jnp.where(lr == 128, 1.0, 0.0)
        g_s[si] = jnp.dot(fm, seln, preferred_element_type=f32, precision=lax.Precision.HIGHEST).astype(bf16).astype(f32)

    for cp in cps[:9]:
        cp.wait()
    wvt_s[...] = _b2u(wqkv_ref[:, 1024:1536].astype(f32).T.astype(bf16))
    rbuf[1] = jnp.zeros((D // 2, 128), u32)
    uraw[...] = jnp.zeros_like(uraw)

    dep = {}

    def tokdep(w):
        if "tok" not in dep or not cfg.get("tok", 0):
            return w
        tok = lax.bitcast_convert_type(dep.pop("tok"), u32)[0:8, 0:128] & zv
        top = _u2b(_b2u(w[0:16, 0:128]) | tok)
        if w.shape[1] > 128:
            top = jnp.concatenate([top, w[0:16, 128:]], axis=1)
        return jnp.concatenate([top, w[16:]], axis=0)

    def adep(v):
        lag = cfg.get("lag", 0)
        h = dep.get("ahist", [])
        if not lag or len(h) < lag:
            return v
        tk = lax.bitcast_convert_type(h[-lag], u32) & zv
        if v.shape[0] != 8:
            tk = jnp.concatenate([tk] * (v.shape[0] // 8), axis=0)
        return lax.bitcast_convert_type(lax.bitcast_convert_type(v, u32) | tk[:, 0:v.shape[1]], f32)

    def seeds_small(c, CHS):
        r0 = _mo(c * CHS, CHS)
        sl = pl.ds(r0, CHS)

        def st_p(s_, val):
            psr[pl.ds(r0 * 8 + s_, CHS, stride=8), :] = val[0]
            psi[pl.ds(r0 * 8 + s_, CHS, stride=8), :] = val[1]

        def st_x(a, val):
            xsr[a // 8, pl.ds(r0 * 8 + a % 8, CHS, stride=8), :] = val[0]
            xsn[a // 8, pl.ds(r0 * 8 + a % 8, CHS, stride=8), :] = -val[1]

        def start():
            dt = adep(_acc_exp(ldt[sl, :].astype(f32)).astype(bf16).astype(f32))
            zr = dt * are[sl, :].astype(f32)
            zi = dt * aim[sl, :].astype(f32)

            def direct(l):
                mag = jnp.exp(zr * l)
                s_, c_ = _sincos(zi * l)
                return mag * c_, mag * s_
            return dt, direct
        dt, direct = start()
        one = (jnp.ones((CHS, N), f32), jnp.zeros((CHS, N), f32))
        st_p(0, one)
        p1 = direct(1.0); st_p(1, p1)
        p2 = _csq(p1); st_p(2, p2)
        p3 = _cmul(p2, p1); st_p(3, p3)
        p4 = _csq(p2); st_p(4, p4)
        st_p(5, _cmul(p4, p1)); st_p(6, _cmul(p4, p2)); p7 = _cmul(p4, p3); st_p(7, p7)
        dep["tok"] = p7[0]
        yield
        dt, direct = start()
        R = {1: direct(8.0)}
        rr[0, sl, :] = R[1][0]; ri[0, sl, :] = R[1][1]
        for k in range(2, 16):
            h = 1 << (k.bit_length() - 1)
            R[k] = _csq(R[h // 2]) if k == h else _cmul(R[h], R[k - h])
            rr[k - 1, sl, :] = R[k][0]; ri[k - 1, sl, :] = R[k][1]
        dep["tok"] = R[15][0]
        yield
        dt, direct = start()
        dB = (dt * bre[sl, :].astype(f32), dt * bim[sl, :].astype(f32))
        w = _cmul((cre[sl, :].astype(f32), cim[sl, :].astype(f32)), dB)
        Q = {1: direct(128.0)}
        Q[2] = _csq(Q[1]); Q[4] = _csq(Q[2]); Q[8] = _csq(Q[4])
        X = {0: w}
        st_x(0, w)
        for a in range(1, 16):
            h = 1 << (a.bit_length() - 1)
            X[a] = _cmul(X[a - h], Q[h])
            st_x(a, X[a])
        x16v = _cmul(X[8], Q[8])[0]
        x16r[sl, :] = x16v
        dep["tok"] = x16v
        yield

    def seeds_gen(t):
        CHS = cfg.get("chs", 32)
        nsub = CH // CHS
        for sub in range(nsub):
            yield from seeds_small(t * nsub + sub, CHS)

    def chan(d):
        r8 = pl.ds(_mo(d * 8, 8), 8)
        vr = psr[r8, :]
        vi = psi[r8, :]
        ers, eis = [vr], [vi]
        for k in range(1, 16):
            if cfg.get("s0", 0):
                r_r = rr[k - 1, pl.ds(d, 8, stride=0), :]
                r_i_ = ri[k - 1, pl.ds(d, 8, stride=0), :]
            else:
                r_r = jnp.broadcast_to(rr[k - 1, pl.ds(d, 1), :], (8, N))
                r_i_ = jnp.broadcast_to(ri[k - 1, pl.ds(d, 1), :], (8, N))
            er, ei = _cmul((r_r, r_i_), (vr, vi))
            ers.append(er); eis.append(ei)
        et = jnp.concatenate([jnp.concatenate(ers, axis=0), jnp.concatenate(eis, axis=0)], axis=1).astype(bf16)
        xr = jnp.concatenate([xsr[0, r8, :], xsr[1, r8, :]], axis=0)
        xn = jnp.concatenate([xsn[0, r8, :], xsn[1, r8, :]], axis=0)
        x = jnp.concatenate([xr, xn], axis=1).astype(bf16)
        o = lax.dot_general(x, et, NT, preferred_element_type=f32)
        kt[0, r8, :] = o[0:8]
        kt[1, r8, :] = o[8:16]

    def chan_gen(d0, n):
        for k in range(n):
            chan(d0 + k)
            yield

    def uf_gen(m):
        um = u_ref[pl.ds(_mo(m * 128, 128), 128), :]
        U = jnp.dot(fm_s[...], um, preferred_element_type=f32)
        yield
        Pv = uraw[...]
        ur, ui = U[0:128], U[128:256]
        pr, pi_ = Pv[0:128], Pv[128:256]
        tr = jnp.concatenate([ur[0:64] - pi_[0:64], ur[64:128] + pi_[64:128]], axis=0)
        ti = jnp.concatenate([ui[0:64] + pr[0:64], ui[64:128] - pr[64:128]], axis=0)
        utr[m] = tr; utd[m] = ti - tr; uts[m] = tr + ti
        uraw[...] = U
        yield

    lane_v = lax.broadcasted_iota(i32, (256, 128), 1)

    def proj_gen(t):
        r0 = _mo(t * 128, 128)
        h0 = _mo(t * 64, 64)
        xt = x_ref[pl.ds(r0, 128), :]
        for nb in range(8):
            qk = jnp.dot(xt, tokdep(wqkv_ref[:, 128 * nb:128 * nb + 128]), preferred_element_type=f32)
            dep.setdefault("ahist", []).append(qk[0:8])
            if nb < 4:
                q_s[pl.ds(h0, 64), 128 * nb:128 * nb + 128] = _b2u((qk * (0.25 * LOG2E)).astype(bf16))
            else:
                k_s[pl.ds(h0, 64), 128 * (nb - 4):128 * (nb - 4) + 128] = _b2u(qk.astype(bf16))
            yield
        for rb in range(4):
            vt = lax.dot_general(tokdep(_u2b(wvt_s[64 * rb:64 * rb + 64, :])), xt, NT, preferred_element_type=f32)
            dep.setdefault("ahist", []).append(vt[0:8])
            vt_s[0, 64 * rb:64 * rb + 64, pl.ds(r0, 128)] = _b2u(vt.astype(bf16))
            rolled = _b2u(pltpu.roll(vt, 64, 1).astype(bf16))
            if cfg.get("dep", 0) and rb == 3 and "tok" in dep:
                tok = lax.bitcast_convert_type(dep["tok"], u32)
                zer = rbuf[2 + 0 * 0, 0:tok.shape[0], :] if False else zbuf[...]
                rolled = rolled | jnp.concatenate([tok[0:8] & zer, ] * 8, axis=0)
            lane_ = lax.broadcasted_iota(i32, (64, 128), 1)
            if isinstance(t, int):
                pc = max(r0 - 128, 0)
            else:
                pc = pl.multiple_of(jnp.maximum(r0 - 128, 0), 128)
            prev = rbuf[(t + 1) % 2, 64 * rb:64 * rb + 64, :]
            vt_s[1, 64 * rb:64 * rb + 64, pl.ds(pc, 128)] = jnp.where(lane_ < 64, prev, rolled)
            rbuf[t % 2, 64 * rb:64 * rb + 64, :] = rolled
            yield

    mode = cfg.get("l1", "seq")

    def proj_iter(t, ufs):
        dep.clear()
        _interleave(proj_gen(t)); _interleave(seeds_gen(t))
        for m in ufs:
            _interleave(uf_gen(m))

    def proj_body_a(t, carry):
        proj_iter(t, [])
        return carry

    def proj_body_b(t, carry):
        proj_iter(t, [2 * (t - 8), 2 * (t - 8) + 1])
        return carry
    lax.fori_loop(0, 8, proj_body_a, 0)
    for cp in cps[9:12]:
        cp.wait()
    lax.fori_loop(8, 16, proj_body_b, 0)
    vt_s[1, :, pl.ds(S - 128, 128)] = rbuf[1]

    lane = lax.broadcasted_iota(i32, (TQ // 2, 128), 1)
    lane2 = lax.broadcasted_iota(i32, (16, 128), 1)
    sbufs = (sbuf0, sbuf1)
    mbufs = (mbuf0, mbuf1)

    def stage1(un, slot, idx, generic=True):
        I = un // 16
        j = un % 16
        g8 = j // 4
        p4 = j % 4
        l0 = _mo(g8 * 128, 128)
        me = (lane >= 32 * p4) & (lane < 32 * p4 + 16)
        mo = (lane >= 32 * p4 + 16) & (lane < 32 * p4 + 32)
        for half in range(2):
            i = 2 * I + half
            q0h = _mo(i * 32, 32)
            if isinstance(i, int):
                wsh = max(i * 32 - 128, 0); v = min(i, 4)
            else:
                wsh = pl.multiple_of(jnp.maximum(i * 32 - 128, 0), 32); v = jnp.minimum(i, 4)
            q8 = q_s[pl.ds(q0h, 32), pl.ds(l0, 128)]
            zero = jnp.zeros_like(q8)
            qm = _u2b(jnp.concatenate([jnp.where(me, q8, zero), jnp.where(mo, q8, zero)], axis=0))
            k8 = _u2b(k_s[pl.ds(wsh, KW // 2), pl.ds(l0, 128)])
            st = lax.dot_general(k8, qm, NT, preferred_element_type=f32)
            if generic:
                st = st + bias_s[v]
            else:
                st = jnp.concatenate([st[0:64] + bias_s[4, 0:64], st[64:256], st[256:320] + bias_s[4, 256:320]], axis=0)
            sbufs[slot][2 * idx + half] = st
            mbufs[slot][2 * idx + half] = jnp.max(st, axis=0, keepdims=True)

    def stage2(un, slot, idx):
        I = un // 16
        j = un % 16
        vrow = _mo(16 * j, 16)
        if isinstance(I, int):
            wsa = max(I * 128 - W, 0); cp = 1 if I >= 2 else 0
        else:
            wsa = pl.multiple_of(jnp.maximum(I * 128 - W, 0), 128); cp = jnp.where(I >= 2, 1, 0)
        outs = []
        for half in range(2):
            st = sbufs[slot][2 * idx + half]
            m = mbufs[slot][2 * idx + half]
            p = jnp.exp2(st - m)
            l = jnp.sum(p, axis=0, keepdims=True)
            vt = vt_s[0 if half == 0 else cp, pl.ds(vrow, 16), pl.ds(wsa, KW)]
            o = jnp.dot(_u2b(vt), p.astype(bf16), preferred_element_type=f32)
            outs.append(o * (1.0 / l))
        oa, ob = outs
        even = jnp.where(lane2 < 64, oa[0:16], pltpu.roll(ob[0:16], 64, 1))
        odd = jnp.where(lane2 < 64, pltpu.roll(oa[16:32], 64, 1), ob[16:32])
        res = jnp.concatenate([even, odd], axis=0).astype(bf16)
        ot_s[pl.ds(vrow, 16), pl.ds(_mo(I * 128, 128), 128)] = _b2u(res)

    NG = 256 // G

    def half_body(t, slot, generic=True):
        o2 = cfg.get("o2", 0)
        if o2 == 0:
            for g in range(G):
                stage2(t * G + g, slot, g)
                chan(t * 2 * G + 2 * g)
                stage1((t + 1) * G + g, 1 - slot, g, generic)
                chan(t * 2 * G + 2 * g + 1)
        elif o2 == 1:
            for g in range(G):
                stage1((t + 1) * G + g, 1 - slot, g, generic)
            for g in range(G):
                stage2(t * G + g, slot, g)
                chan(t * 2 * G + 2 * g); chan(t * 2 * G + 2 * g + 1)
        elif o2 == 2:
            for g in range(2 * G):
                chanidx = t * 2 * G + g
                chan(chanidx)
            for g in range(G):
                stage2(t * G + g, slot, g)
                stage1((t + 1) * G + g, 1 - slot, g, generic)
        elif o2 == 3:
            for g in range(G):
                stage1((t + 1) * G + g, 1 - slot, g, generic)
                chan(t * 2 * G + 2 * g)
                stage2(t * G + g, slot, g)
                chan(t * 2 * G + 2 * g + 1)

    def attn_body(t2, carry):
        half_body(2 * t2, 0)
        half_body(2 * t2 + 1, 1)
        return carry

    def attn_body_fast(t2, carry):
        half_body(2 * t2, 0, False)
        half_body(2 * t2 + 1, 1, False)
        return carry
    if not cfg.get("n2", 1):
        def cb(t, c):
            for uu in range(8):
                chan(t * 8 + uu)
            return c
        lax.fori_loop(0, 64, cb, 0)
        ot_s[...] = _b2u(_u2b(q_s[...]).T[:512, :]) if False else ot_s[...]
        ot_s[:, 0:512] = k_s[0:256, :] + vt_s[1, :, 0:512] + vt_s[0, :, 0:512]
        ot_s[:, 512:2048] = jnp.zeros((256, 1536), u32) + q_s[0:256, 0:1]
    if cfg.get("n2", 1):
        for g in range(G):
            stage1(g, 0, g)
        ngen = (64 // G) // 2
        lax.fori_loop(0, ngen, attn_body, 0)
        lax.fori_loop(ngen, NG // 2 - 1, attn_body_fast, 0)
        half_body(NG - 2, 0, False)
        for g in range(G):
            stage2((NG - 1) * G + g, (NG - 1) % 2, g)
            chan((NG - 1) * 2 * G + 2 * g)
            chan((NG - 1) * 2 * G + 2 * g + 1)

    if not cfg.get("n3", 1):
        out_ref[...] = jnp.zeros_like(out_ref)
        cps[-1].wait()
        oc = pltpu.make_async_copy(out_ref, out_h, osem.at[0]); oc.start(); oc.wait()
        return

    cps[-1].wait()
    out_ref[:, 0:D] = lax.dot_general(_u2b(ot_s[...]), wo_ref[...], TN, preferred_element_type=f32).astype(out_ref.dtype)
    ocpA = pltpu.make_async_copy(out_ref.at[:, 0:D], out_h.at[:, 0:D], osem.at[NB])
    ocpA.start()

    ones8 = jnp.ones((8, 128), bf16)
    nf0 = lax.dot_general(ones8, x16r[...].astype(bf16), NT, preferred_element_type=f32)

    def kf_body(tt, nf):
        i = 15 - tt
        si = jnp.where(i < 2, 0, jnp.where(i < 4, 1, jnp.where(i < 8, 2, 3)))
        ktv = kt[i >> 3, pl.ds(i & 7, D, stride=8), :]
        R = lax.dot_general(fa_s[si], ktv.astype(bf16), NT, preferred_element_type=f32)
        g_ = g_s[si]
        kf = R[0:256] + jnp.concatenate([g_, g_, g_, g_], axis=1) * nf[0:1, :]
        kfr[i] = kf[0:128]; kfi[i] = kf[128:256]; kfs[i] = kf[0:128] + kf[128:256]
        return jnp.broadcast_to(R[256:257, :], (8, D))
    lax.fori_loop(0, NB, kf_body, nf0)

    def pr_body(p, carry):
        g_ = p // 4
        cc = p % 4
        rs = pl.ds(pl.multiple_of(g_ * 8, 8), 8)
        ls = pl.ds(pl.multiple_of(cc * 128, 128), 128)
        K = [(kfr[i, rs, ls], kfi[i, rs, ls], kfs[i, rs, ls]) for i in range(NB)]
        U = [(utr[m, rs, ls], utd[m, rs, ls], uts[m, rs, ls]) for m in range(NB)]
        for j in range(NB):
            a1 = a2 = a3 = None
            for i in range(j + 1):
                kr, ki, ks = K[i]
                ur, ud, us = U[j - i]
                t1 = ur * ks; t2 = kr * ud; t3 = ki * us
                a1 = t1 if a1 is None else a1 + t1
                a2 = t2 if a2 is None else a2 + t2
                a3 = t3 if a3 is None else a3 + t3
            zb[j, rs, ls] = a1 - a3
            zb[j, pl.ds(pl.multiple_of(128 + g_ * 8, 8), 8), ls] = a1 + a2
        return carry
    lax.fori_loop(0, 64, pr_body, 0)

    def inv_body(j, carry):
        z = zb[j].astype(bf16)
        y = jnp.dot(gm_s[...], z, preferred_element_type=f32)
        rs = pl.ds(pl.multiple_of(j * 128, 128), 128)
        out_ref[rs, D:2 * D] = (y + u_ref[rs, :].astype(f32) * dsk[...].astype(f32)).astype(out_ref.dtype)
        pltpu.make_async_copy(out_ref.at[rs, D:2 * D], out_h.at[rs, D:2 * D], osem.at[j]).start()
        return carry
    lax.fori_loop(0, NB, inv_body, 0)
    for j in range(NB):
        pltpu.make_async_copy(out_ref.at[pl.ds(j * 128, 128), D:2 * D], out_h.at[pl.ds(j * 128, 128), D:2 * D], osem.at[j]).wait()
    ocpA.wait()


_CFG = {"l1": "seq", "s0": 1, "o2": 3}


def build(cfg):
    @jax.jit
    def pallas_concat_heads__sliding_block__ssm_conv_s4__prompt_kernel(
        A_x, A_wqkv, A_wo, B_u, B_A_re, B_A_im, B_B_re, B_B_im, B_C_re, B_C_im, B_log_dt, B_Dskip,
    ):
        out = pl.pallas_call(
            functools.partial(_kernel, cfg=cfg),
            out_shape=jax.ShapeDtypeStruct((S, 2 * D), bf16),
            in_specs=[pl.BlockSpec(memory_space=pl.ANY)] * 12,
            out_specs=pl.BlockSpec(memory_space=pl.ANY),
            scratch_shapes=[
                pltpu.VMEM((S, D), bf16), pltpu.VMEM((D, 3 * D), bf16), pltpu.VMEM((D, D), bf16), pltpu.VMEM((S, D), bf16),
                pltpu.VMEM((D, N), bf16), pltpu.VMEM((D, N), bf16), pltpu.VMEM((D, N), bf16),
                pltpu.VMEM((D, N), bf16), pltpu.VMEM((D, N), bf16), pltpu.VMEM((D, N), bf16),
                pltpu.VMEM((D, 1), bf16), pltpu.VMEM((1, D), bf16), pltpu.VMEM((S, 2 * D), bf16),
                pltpu.SemaphoreType.DMA((13,)), pltpu.SemaphoreType.DMA((NB + 1,)),
                pltpu.VMEM((S // 2, D), u32),
                pltpu.VMEM((S // 2, D), u32),
                pltpu.VMEM((2, D // 2, S), u32),
                pltpu.VMEM((D // 2, S), u32),
                pltpu.VMEM((5, KW, 128), f32),
                pltpu.VMEM((2, D // 2, 128), u32),
                pltpu.VMEM((2 * G, KW, 128), f32), pltpu.VMEM((2 * G, 1, 128), f32),
                pltpu.VMEM((2 * G, KW, 128), f32), pltpu.VMEM((2 * G, 1, 128), f32),
                pltpu.VMEM((D // 2, D), u32),
                pltpu.VMEM((D * 8, N), f32), pltpu.VMEM((D * 8, N), f32),
                pltpu.VMEM((15, D, N), f32), pltpu.VMEM((15, D, N), f32),
                pltpu.VMEM((2, D * 8, N), f32), pltpu.VMEM((2, D * 8, N), f32),
                pltpu.VMEM((D, N), f32),
                pltpu.VMEM((2, D * 8, 128), f32),
                pltpu.VMEM((256, 128), bf16), pltpu.VMEM((128, 256), bf16),
                pltpu.VMEM((4, 272, 128), bf16), pltpu.VMEM((4, 256, 128), f32),
                pltpu.VMEM((NB, 128, D), f32), pltpu.VMEM((NB, 128, D), f32), pltpu.VMEM((NB, 128, D), f32),
                pltpu.VMEM((NB, 128, D), f32), pltpu.VMEM((NB, 128, D), f32), pltpu.VMEM((NB, 128, D), f32),
                pltpu.VMEM((256, D), f32),
                pltpu.VMEM((NB, 256, D), f32),
                pltpu.VMEM((8, 128), u32),
                pltpu.SemaphoreType.REGULAR,
            ],
            compiler_params=pltpu.CompilerParams(vmem_limit_bytes=120 * 1024 * 1024),
        )(
            A_x.reshape(S, D), A_wqkv, A_wo, B_u.reshape(S, D),
            B_A_re, B_A_im, B_B_re, B_B_im, B_C_re, B_C_im,
            B_log_dt.reshape(D, 1), B_Dskip.reshape(1, D),
        )
        return out.reshape(1, S, 2 * D)
    return pallas_concat_heads__sliding_block__ssm_conv_s4__prompt_kernel


pallas_concat_heads__sliding_block__ssm_conv_s4__prompt_kernel = build(_CFG)
```

```python
import math

import jax
import jax.numpy as jnp
from jax import lax
from jax.experimental import pallas as pl
from jax.experimental.pallas import tpu as pltpu

f32 = jnp.float32
bf16 = jnp.bfloat16
u32 = jnp.uint32
i32 = jnp.int32

S = 2048
D = 512
W = 256
TQ = 64
KW = 320
N = 128
NB = 16
G = 8
CH = 32
UQ = 4
UP = 4
UK = 16
LOG2E = 1.4426950408889634
NEG = -1e9
NT = (((1,), (1,)), ((), ()))


def _b2u(x):
    return pltpu.bitcast(x, u32)


def _u2b(x):
    return pltpu.bitcast(x, bf16)


def _mo(x, m):
    return x if isinstance(x, int) else pl.multiple_of(x, m)


def _cmul(a, b):
    ar, ai = a
    br, bi = b
    return ar * br - ai * bi, ar * bi + ai * br


def _csq(a):
    ar, ai = a
    return ar * ar - ai * ai, (ar + ar) * ai


def _sincos(th):
    n = jnp.round(th * 0.6366197723675814)
    r = ((th - n * 1.5703125) - n * 4.837512969970703e-04) - n * 7.549789948768648e-08
    r2 = r * r
    s = r + r * r2 * (-1.6666654611e-1 + r2 * (8.3321608736e-3 + r2 * (-1.9515295891e-4)))
    c = 1.0 + r2 * (-0.5 + r2 * (4.166664568298827e-2 + r2 * (-1.388731625493765e-3 + r2 * 2.443315711809948e-5)))
    q = n.astype(i32)
    swap = (q & 1) == 1
    ss = jnp.where(swap, c, s)
    cc = jnp.where(swap, s, c)
    ss = jnp.where((q & 2) == 2, -ss, ss)
    cc = jnp.where(((q + 1) & 2) == 2, -cc, cc)
    return ss, cc


def _acc_exp(x):
    x = jnp.clip(x, -87.0, 88.0)
    n = jnp.round(x * 1.4426950408889634)
    r = (x - n * 0.693359375) - n * (-2.12194440e-4)
    p = 1.0 + r * (1.0 + r * (0.5 + r * (1.6666667163e-1 + r * (4.1666667908e-2 + r * (
        8.3333337680e-3 + r * (1.3888889225e-3 + r * 1.9841270114e-4))))))
    e = lax.bitcast_convert_type((n.astype(i32) + 127) << 23, f32)
    return p * e


def _kernel(x_h, wqkv_h, wo_h, u_h, are_h, aim_h, bre_h, bim_h, cre_h, cim_h, ldt_h, dsk_h, out_h,
            x_ref, wqkv_ref, wo_ref, u_ref, are, aim, bre, bim, cre, cim, ldt, dsk, out_ref, dsem, osem,
            dtc,
            q_s, k_s, vt_s, ot_s, bias_s, rbuf, sbuf0, mbuf0, sbuf1, mbuf1, wvt_s,
            psr, psi, rr, ri, xsr, xsn, x16r, kt,
            fm_s, gm_s, fa_s, g_s, kfr, kfi, kfs, utr, utd, uts, uraw, zb):
    srcs = [wqkv_h, ldt_h, are_h, aim_h, bre_h, bim_h, cre_h, cim_h,
            x_h.at[0:S // 2], x_h.at[S // 2:S], u_h, dsk_h, wo_h]
    dsts = [wqkv_ref, ldt, are, aim, bre, bim, cre, cim,
            x_ref.at[0:S // 2], x_ref.at[S // 2:S], u_ref, dsk, wo_ref]
    cps = [pltpu.make_async_copy(a, b, dsem.at[k]) for k, (a, b) in enumerate(zip(srcs, dsts))]
    for cp in cps:
        cp.start()

    kk = lax.broadcasted_iota(i32, (KW, 128), 0)
    qq = lax.broadcasted_iota(i32, (KW, 128), 1) % TQ
    for v in range(4):
        bias_s[v] = jnp.where(kk <= qq + TQ * v, 0.0, NEG).astype(f32)
    bias_s[4] = jnp.where((kk > qq) & (kk <= qq + W), 0.0, NEG).astype(f32)

    r_i = lax.broadcasted_iota(i32, (128, 128), 0)
    t_i = lax.broadcasted_iota(i32, (128, 128), 1)
    fr = jnp.where(r_i < 64, 2 * r_i, 2 * (r_i - 64) + 1)
    th = (((2 * fr + 1) * t_i) & 511).astype(f32) * (math.pi / 256.0)
    fm = jnp.concatenate([jnp.cos(th), -jnp.sin(th)], axis=0)
    fm_s[...] = fm.astype(bf16)
    fr2 = jnp.where(t_i < 64, 2 * t_i, 2 * (t_i - 64) + 1)
    th2 = (((2 * fr2 + 1) * r_i) & 511).astype(f32) * (math.pi / 256.0)
    gm_s[...] = (jnp.concatenate([jnp.cos(th2), -jnp.sin(th2)], axis=1).astype(bf16).astype(f32)
                 * (1.0 / 128.0)).astype(bf16)
    e0 = jnp.where((lax.broadcasted_iota(i32, (16, 128), 0) == 0)
                   & (lax.broadcasted_iota(i32, (16, 128), 1) == 0), 1.0, 0.0)
    fa_s[0] = jnp.concatenate([fm, e0], axis=0).astype(bf16)
    g_s[0] = jnp.zeros((256, 128), f32)
    for si, i0 in ((1, 2), (2, 4), (3, 8)):
        lag = (128 * i0 + r_i).astype(f32)
        lr = lag.astype(bf16).astype(f32).astype(i32) - 128 * i0
        sel = jnp.where(lr == t_i, 1.0, 0.0)
        fp = jnp.dot(fm, sel, preferred_element_type=f32, precision=lax.Precision.HIGHEST)
        fa_s[si] = jnp.concatenate([fp, e0], axis=0).astype(bf16)
        seln = jnp.where(lr == 128, 1.0, 0.0)
        g_s[si] = jnp.dot(fm, seln, preferred_element_type=f32,
                          precision=lax.Precision.HIGHEST).astype(bf16).astype(f32)

    for cp in cps[:9]:
        cp.wait()
    wvt_s[...] = _b2u(wqkv_ref[:, 1024:1536].astype(f32).T.astype(bf16))
    dt_row = _acc_exp(ldt[...].astype(f32).reshape(1, D)).astype(bf16).astype(f32)
    dtc[...] = jnp.broadcast_to(dt_row, (8, D)).T[:, 0:1]
    rbuf[1] = jnp.zeros((D // 2, 128), u32)
    uraw[...] = jnp.zeros_like(uraw)

    def seeds(c):
        r0 = _mo(c * CH, CH)
        sl = pl.ds(r0, CH)
        dt = dtc[sl, :]
        zr = dt * are[sl, :].astype(f32)
        zi = dt * aim[sl, :].astype(f32)

        def direct(l):
            mag = jnp.exp(zr * l)
            s_, c_ = _sincos(zi * l)
            return mag * c_, mag * s_

        def st_p(s_, val):
            psr[pl.ds(r0 * 8 + s_, CH, stride=8), :] = val[0]
            psi[pl.ds(r0 * 8 + s_, CH, stride=8), :] = val[1]

        def st_x(a, val):
            xsr[a // 8, pl.ds(r0 * 8 + a % 8, CH, stride=8), :] = val[0]
            xsn[a // 8, pl.ds(r0 * 8 + a % 8, CH, stride=8), :] = -val[1]

        st_p(0, (jnp.ones((CH, N), f32), jnp.zeros((CH, N), f32)))
        p1 = direct(1.0); st_p(1, p1)
        p2 = _csq(p1); st_p(2, p2)
        p3 = _cmul(p2, p1); st_p(3, p3)
        p4 = _csq(p2); st_p(4, p4)
        st_p(5, _cmul(p4, p1)); st_p(6, _cmul(p4, p2)); st_p(7, _cmul(p4, p3))
        R = {1: direct(8.0)}
        rr[0, sl, :] = R[1][0]; ri[0, sl, :] = R[1][1]
        for k in range(2, 16):
            h = 1 << (k.bit_length() - 1)
            R[k] = _csq(R[h // 2]) if k == h else _cmul(R[h], R[k - h])
            rr[k - 1, sl, :] = R[k][0]; ri[k - 1, sl, :] = R[k][1]
        dB = (dt * bre[sl, :].astype(f32), dt * bim[sl, :].astype(f32))
        w = _cmul((cre[sl, :].astype(f32), cim[sl, :].astype(f32)), dB)
        Q = {1: direct(128.0)}
        Q[2] = _csq(Q[1]); Q[4] = _csq(Q[2]); Q[8] = _csq(Q[4])
        X = {0: w}
        st_x(0, w)
        for a in range(1, 16):
            h = 1 << (a.bit_length() - 1)
            X[a] = _cmul(X[a - h], Q[h])
            st_x(a, X[a])
        x16r[sl, :] = _cmul(X[8], Q[8])[0]

    def chan(d):
        r8 = pl.ds(_mo(d * 8, 8), 8)
        vr = psr[r8, :]
        vi = psi[r8, :]
        ers, eis = [vr], [vi]
        for k in range(1, 16):
            r_r = jnp.broadcast_to(rr[k - 1, pl.ds(d, 1), :], (8, N))
            r_i_ = jnp.broadcast_to(ri[k - 1, pl.ds(d, 1), :], (8, N))
            er, ei = _cmul((r_r, r_i_), (vr, vi))
            ers.append(er); eis.append(ei)
        et = jnp.concatenate([jnp.concatenate(ers, axis=0), jnp.concatenate(eis, axis=0)], axis=1).astype(bf16)
        xr = jnp.concatenate([xsr[0, r8, :], xsr[1, r8, :]], axis=0)
        xn = jnp.concatenate([xsn[0, r8, :], xsn[1, r8, :]], axis=0)
        x = jnp.concatenate([xr, xn], axis=1).astype(bf16)
        o = lax.dot_general(x, et, NT, preferred_element_type=f32)
        kt[0, r8, :] = o[0:8]
        kt[1, r8, :] = o[8:16]

    def uf(m):
        um = u_ref[pl.ds(_mo(m * 128, 128), 128), :]
        U = jnp.dot(fm_s[...], um, preferred_element_type=f32)
        Pv = uraw[...]
        ur, ui = U[0:128], U[128:256]
        pr, pi_ = Pv[0:128], Pv[128:256]
        tr = jnp.concatenate([ur[0:64] - pi_[0:64], ur[64:128] + pi_[64:128]], axis=0)
        ti = jnp.concatenate([ui[0:64] + pr[0:64], ui[64:128] - pr[64:128]], axis=0)
        utr[m] = tr; utd[m] = ti - tr; uts[m] = tr + ti
        uraw[...] = U

    lane64 = lax.broadcasted_iota(i32, (64, 128), 1)

    def proj(t):
        r0 = _mo(t * 128, 128)
        h0 = _mo(t * 64, 64)
        xt = x_ref[pl.ds(r0, 128), :]
        for nb in range(8):
            qk = jnp.dot(xt, wqkv_ref[:, 128 * nb:128 * nb + 128], preferred_element_type=f32)
            if nb < 4:
                q_s[pl.ds(h0, 64), 128 * nb:128 * nb + 128] = _b2u((qk * (0.25 * LOG2E)).astype(bf16))
            else:
                k_s[pl.ds(h0, 64), 128 * (nb - 4):128 * (nb - 4) + 128] = _b2u(qk.astype(bf16))
        for rb in range(4):
            rs = slice(64 * rb, 64 * rb + 64)
            vt = lax.dot_general(_u2b(wvt_s[rs, :]), xt, NT, preferred_element_type=f32)
            vt_s[0, rs, pl.ds(r0, 128)] = _b2u(vt.astype(bf16))
            rolled = _b2u(pltpu.roll(vt, 64, 1).astype(bf16))
            pc = pl.multiple_of(jnp.maximum(r0 - 128, 0), 128)
            prev = rbuf[(t + 1) % 2, rs, :]
            vt_s[1, rs, pl.ds(pc, 128)] = jnp.where(lane64 < 64, prev, rolled)
            rbuf[t % 2, rs, :] = rolled

    def proj_body_a(tt, carry):
        for k in range(UP):
            t = tt * UP + k
            proj(t); seeds(t)
        return carry

    def proj_body_b(tt, carry):
        for k in range(UP):
            t = tt * UP + k
            proj(t); seeds(t)
            uf(2 * (t - 8)); uf(2 * (t - 8) + 1)
        return carry
    lax.fori_loop(0, 8 // UP, proj_body_a, 0)
    for cp in cps[9:12]:
        cp.wait()
    lax.fori_loop(8 // UP, 16 // UP, proj_body_b, 0)
    vt_s[1, :, pl.ds(S - 128, 128)] = rbuf[1]

    lane = lax.broadcasted_iota(i32, (TQ // 2, 128), 1)
    lane2 = lax.broadcasted_iota(i32, (16, 128), 1)
    sbufs = (sbuf0, sbuf1)
    mbufs = (mbuf0, mbuf1)

    def stage1(un, slot, idx, generic):
        I = un // 16
        j = un % 16
        l0 = _mo((j // 4) * 128, 128)
        p4 = j % 4
        me = (lane >= 32 * p4) & (lane < 32 * p4 + 16)
        mo = (lane >= 32 * p4 + 16) & (lane < 32 * p4 + 32)
        for half in range(2):
            i = 2 * I + half
            q0h = _mo(i * 32, 32)
            if isinstance(i, int):
                wsh = max(i * 32 - 128, 0); v = min(i, 4)
            else:
                wsh = pl.multiple_of(jnp.maximum(i * 32 - 128, 0), 32); v = jnp.minimum(i, 4)
            q8 = q_s[pl.ds(q0h, 32), pl.ds(l0, 128)]
            zero = jnp.zeros_like(q8)
            qm = _u2b(jnp.concatenate([jnp.where(me, q8, zero), jnp.where(mo, q8, zero)], axis=0))
            k8 = _u2b(k_s[pl.ds(wsh, KW // 2), pl.ds(l0, 128)])
            st = lax.dot_general(k8, qm, NT, preferred_element_type=f32)
            if generic:
                st = st + bias_s[v]
            else:
                st = jnp.concatenate([st[0:64] + bias_s[4, 0:64], st[64:256], st[256:320] + bias_s[4, 256:320]],
                                     axis=0)
            sbufs[slot][2 * idx + half] = st
            mbufs[slot][2 * idx + half] = jnp.max(st, axis=0, keepdims=True)

    def stage2(un, slot, idx):
        I = un // 16
        j = un % 16
        vrow = _mo(16 * j, 16)
        if isinstance(I, int):
            wsa = max(I * 128 - W, 0); cp = 1 if I >= 2 else 0
        else:
            wsa = pl.multiple_of(jnp.maximum(I * 128 - W, 0), 128); cp = jnp.where(I >= 2, 1, 0)
        outs = []
        for half in range(2):
            st = sbufs[slot][2 * idx + half]
            m = mbufs[slot][2 * idx + half]
            p = jnp.exp2(st - m)
            l = jnp.sum(p, axis=0, keepdims=True)
            vt = vt_s[0 if half == 0 else cp, pl.ds(vrow, 16), pl.ds(wsa, KW)]
            o = jnp.dot(_u2b(vt), p.astype(bf16), preferred_element_type=f32)
            outs.append(o * (1.0 / l))
        oa, ob = outs
        even = jnp.where(lane2 < 64, oa[0:16], pltpu.roll(ob[0:16], 64, 1))
        odd = jnp.where(lane2 < 64, pltpu.roll(oa[16:32], 64, 1), ob[16:32])
        res = jnp.concatenate([even, odd], axis=0).astype(bf16)
        ot_s[pl.ds(vrow, 16), pl.ds(_mo(I * 128, 128), 128)] = _b2u(res)

    NG = 256 // G

    def half_body(t, slot, generic):
        for g in range(G):
            stage1((t + 1) * G + g, 1 - slot, g, generic)
            chan(t * 2 * G + 2 * g)
            stage2(t * G + g, slot, g)
            chan(t * 2 * G + 2 * g + 1)

    def attn_generic(t2, carry):
        half_body(2 * t2, 0, True)
        half_body(2 * t2 + 1, 1, True)
        return carry

    def attn_fast(t4, carry):
        for k in range(4):
            half_body(4 * t4 + k, k % 2, False)
        return carry
    for g in range(G):
        stage1(g, 0, g, True)
    lax.fori_loop(0, 2, attn_generic, 0)
    lax.fori_loop(1, 7, attn_fast, 0)
    for t in range(28, 31):
        half_body(t, t % 2, False)
    for g in range(G):
        stage2((NG - 1) * G + g, (NG - 1) % 2, g)
        chan((NG - 1) * 2 * G + 2 * g)
        chan((NG - 1) * 2 * G + 2 * g + 1)

    cps[-1].wait()
    out_ref[:, 0:D] = lax.dot_general(_u2b(ot_s[...]), wo_ref[...], (((0,), (0,)), ((), ())),
                                      preferred_element_type=f32).astype(out_ref.dtype)
    ocpA = pltpu.make_async_copy(out_ref.at[:, 0:D], out_h.at[:, 0:D], osem.at[NB])
    ocpA.start()

    ones8 = jnp.ones((8, 128), bf16)
    nf0 = lax.dot_general(ones8, x16r[...].astype(bf16), NT, preferred_element_type=f32)

    def kf_one(i, nf):
        si = jnp.where(i < 2, 0, jnp.where(i < 4, 1, jnp.where(i < 8, 2, 3)))
        ktv = kt[i >> 3, pl.ds(i & 7, D, stride=8), :]
        R = lax.dot_general(fa_s[si], ktv.astype(bf16), NT, preferred_element_type=f32)
        g_ = g_s[si]
        kf = R[0:256] + jnp.concatenate([g_, g_, g_, g_], axis=1) * nf[0:1, :]
        kfr[i] = kf[0:128]; kfi[i] = kf[128:256]; kfs[i] = kf[0:128] + kf[128:256]
        return jnp.broadcast_to(R[256:257, :], (8, D))

    def kf_body(tt, nf):
        for k in range(UK):
            nf = kf_one(15 - (tt * UK + k), nf)
        return nf
    lax.fori_loop(0, NB // UK, kf_body, nf0)

    def pr_one(p):
        g_ = p // 4
        cc = p % 4
        rs = pl.ds(pl.multiple_of(g_ * 8, 8), 8)
        ls = pl.ds(pl.multiple_of(cc * 128, 128), 128)
        K = [(kfr[i, rs, ls], kfi[i, rs, ls], kfs[i, rs, ls]) for i in range(NB)]
        U = [(utr[m, rs, ls], utd[m, rs, ls], uts[m, rs, ls]) for m in range(NB)]
        for j in range(NB):
            a1 = a2 = a3 = None
            for i in range(j + 1):
                kr, ki, ks = K[i]
                ur, ud, us = U[j - i]
                t1 = ur * ks; t2 = kr * ud; t3 = ki * us
                a1 = t1 if a1 is None else a1 + t1
                a2 = t2 if a2 is None else a2 + t2
                a3 = t3 if a3 is None else a3 + t3
            zb[j, rs, ls] = a1 - a3
            zb[j, pl.ds(pl.multiple_of(128 + g_ * 8, 8), 8), ls] = a1 + a2

    def pr_body(pp, carry):
        for k in range(UQ):
            pr_one(pp * UQ + k)
        return carry
    lax.fori_loop(0, 64 // UQ, pr_body, 0)

    def inv_body(jj, carry):
        for k in range(UK):
            j = jj * UK + k
            z = zb[j].astype(bf16)
            y = jnp.dot(gm_s[...], z, preferred_element_type=f32)
            rs = pl.ds(pl.multiple_of(j * 128, 128), 128)
            out_ref[rs, D:2 * D] = (y + u_ref[rs, :].astype(f32) * dsk[...].astype(f32).reshape(1, D)).astype(out_ref.dtype)
            pltpu.make_async_copy(out_ref.at[rs, D:2 * D], out_h.at[rs, D:2 * D], osem.at[j]).start()
        return carry
    lax.fori_loop(0, NB // UK, inv_body, 0)
    for j in range(NB):
        pltpu.make_async_copy(out_ref.at[pl.ds(j * 128, 128), D:2 * D],
                              out_h.at[pl.ds(j * 128, 128), D:2 * D], osem.at[j]).wait()
    ocpA.wait()


@jax.jit
def pallas_concat_heads__sliding_block__ssm_conv_s4__prompt_kernel(
    A_x: jax.Array,
    A_wqkv: jax.Array,
    A_wo: jax.Array,
    B_u: jax.Array,
    B_A_re: jax.Array,
    B_A_im: jax.Array,
    B_B_re: jax.Array,
    B_B_im: jax.Array,
    B_C_re: jax.Array,
    B_C_im: jax.Array,
    B_log_dt: jax.Array,
    B_Dskip: jax.Array,
):
    out = pl.pallas_call(
        _kernel,
        out_shape=jax.ShapeDtypeStruct((S, 2 * D), bf16),
        in_specs=[pl.BlockSpec(memory_space=pl.ANY)] * 12,
        out_specs=pl.BlockSpec(memory_space=pl.ANY),
        scratch_shapes=[
            pltpu.VMEM((S, D), bf16), pltpu.VMEM((D, 3 * D), bf16), pltpu.VMEM((D, D), bf16), pltpu.VMEM((S, D), bf16),
            pltpu.VMEM((D, N), bf16), pltpu.VMEM((D, N), bf16), pltpu.VMEM((D, N), bf16),
            pltpu.VMEM((D, N), bf16), pltpu.VMEM((D, N), bf16), pltpu.VMEM((D, N), bf16),
            pltpu.VMEM((D,), bf16), pltpu.VMEM((D,), bf16), pltpu.VMEM((S, 2 * D), bf16),
            pltpu.SemaphoreType.DMA((13,)), pltpu.SemaphoreType.DMA((NB + 1,)),
            pltpu.VMEM((D, 1), f32),
            pltpu.VMEM((S // 2, D), u32),
            pltpu.VMEM((S // 2, D), u32),
            pltpu.VMEM((2, D // 2, S), u32),
            pltpu.VMEM((D // 2, S), u32),
            pltpu.VMEM((5, KW, 128), f32),
            pltpu.VMEM((2, D // 2, 128), u32),
            pltpu.VMEM((2 * G, KW, 128), f32), pltpu.VMEM((2 * G, 1, 128), f32),
            pltpu.VMEM((2 * G, KW, 128), f32), pltpu.VMEM((2 * G, 1, 128), f32),
            pltpu.VMEM((D // 2, D), u32),
            pltpu.VMEM((D * 8, N), f32), pltpu.VMEM((D * 8, N), f32),
            pltpu.VMEM((15, D, N), f32), pltpu.VMEM((15, D, N), f32),
            pltpu.VMEM((2, D * 8, N), f32), pltpu.VMEM((2, D * 8, N), f32),
            pltpu.VMEM((D, N), f32),
            pltpu.VMEM((2, D * 8, 128), f32),
            pltpu.VMEM((256, 128), bf16), pltpu.VMEM((128, 256), bf16),
            pltpu.VMEM((4, 272, 128), bf16), pltpu.VMEM((4, 256, 128), f32),
            pltpu.VMEM((NB, 128, D), f32), pltpu.VMEM((NB, 128, D), f32), pltpu.VMEM((NB, 128, D), f32),
            pltpu.VMEM((NB, 128, D), f32), pltpu.VMEM((NB, 128, D), f32), pltpu.VMEM((NB, 128, D), f32),
            pltpu.VMEM((256, D), f32),
            pltpu.VMEM((NB, 256, D), f32),
        ],
        compiler_params=pltpu.CompilerParams(vmem_limit_bytes=120 * 1024 * 1024),
    )(
        A_x.reshape(S, D), A_wqkv, A_wo, B_u.reshape(S, D),
        B_A_re, B_A_im, B_B_re, B_B_im, B_C_re, B_C_im,
        B_log_dt, B_Dskip,
    )
    return out.reshape(1, S, 2 * D)
```
